```python
import os as _os
_os.environ.setdefault("JAX_PLATFORMS", "cpu")
import jax
import jax.numpy as jnp

def _softmax(x, axis=-1):
    return jax.nn.softmax(x, axis=axis)
def _gelu(x):
    return jax.nn.gelu(x, approximate=True)
def _silu(x):
    return jax.nn.silu(x)
def _sigmoid(x):
    return jax.nn.sigmoid(x)
def _layernorm(x, axis=-1, eps=1e-5):
    m = jnp.mean(x, axis=axis, keepdims=True)
    v = jnp.var(x, axis=axis, keepdims=True)
    return (x - m) / jnp.sqrt(v + eps)
def _scatter_add(tgt, idx, src, axis=0):
    return tgt.at[idx].add(src)
def _segment_sum(src, seg, n):
    return jax.ops.segment_sum(src, seg, n)
class _Rng:
    def __init__(self, key):
        self._k = key
    def _next(self):
        self._k, sub = jax.random.split(self._k)
        return sub
    def normal(self, shape):
        return jax.random.normal(self._next(), shape, dtype=jnp.bfloat16)
    def randint(self, lo, hi, shape):
        return jax.random.randint(self._next(), shape, lo, hi, dtype=jnp.int32)
    def uniform(self, shape, lo=0.0, hi=1.0):
        return jax.random.uniform(self._next(), shape, jnp.bfloat16, lo, hi)
    def permutation(self, n):
        return jax.random.permutation(self._next(), n)


kernel_name = 'sequential_preLN__sliding_local_dilated__dense_activation_silu__prompt'

def setup_inputs():
    _rng = _Rng(jax.random.key(int.from_bytes(__import__("os").urandom(4), "little")))
    _w = (lambda a: (lambda t: t.astype(jnp.bfloat16) if jnp.issubdtype(t.dtype, jnp.floating) else t)(jnp.asarray(a)))
    def _A_setup():
        B, S, D = 1, 2048, 1024
        return {
            "x": _w((lambda *s: _rng.normal(s) * 0.05)(B, S, D)),
            "wqkv": _w((lambda *s: _rng.normal(s) * 0.05)(D, 3 * D)),
            "wo": _w((lambda *s: _rng.normal(s) * 0.05)(D, D)),
        }
    _A_in = _A_setup()

    def _B_setup():
        B, S, D, F = 1, 2048, 1024, 3584
        return {
            "x": _w((lambda *s: _rng.normal(s) * 0.05)(B, S, D)),
            "w1": _w((lambda *s: _rng.normal(s) * 0.05)(D, F) * (D ** -0.5)),
            "w2": _w((lambda *s: _rng.normal(s) * 0.05)(F, D) * (F ** -0.5)),
        }
    _B_in = _B_setup()

    return {
        "A_x": _A_in["x"],
        "A_wqkv": _A_in["wqkv"],
        "A_wo": _A_in["wo"],
        "B_x": _B_in["x"],
        "B_w1": _B_in["w1"],
        "B_w2": _B_in["w2"],
    }

def reference(A_x, A_wqkv, A_wo, B_x, B_w1, B_w2):
    def _A_ref(x, wqkv, wo):
        B, S, D = x.shape
        H = 32; Dh = D // H
        W, dil = 8, 2
        qkv = (lambda x, *d: x.transpose(*d))((x @ wqkv).reshape(B, S, 3, H, Dh), 2, 0, 3, 1, 4)
        q, k, v = qkv[0], qkv[1], qkv[2]
        scale = Dh ** -0.5
        pos = jnp.arange(S)
        off = jnp.arange(W) * dil
        idx = pos[:, None] - off[None, :]
        mask = idx >= 0
        idx_c = jnp.where(mask, idx, 0).reshape(-1)
        kg = k[:, :, idx_c, :].reshape(B, H, S, W, Dh)
        vg = v[:, :, idx_c, :].reshape(B, H, S, W, Dh)
        logits = jnp.einsum("bhsd,bhswd->bhsw", q, kg) * scale
        logits = jnp.where(mask[None, None, :, :], logits, -1e9)
        attn = _softmax(logits, axis=-1)
        o = jnp.einsum("bhsw,bhswd->bhsd", attn, vg)
        return (lambda x, *d: x.transpose(*d))(o, 0, 2, 1, 3).reshape(B, S, D) @ wo

    def _B_ref(x, w1, w2):
        h = jnp.einsum("bsd,df->bsf", x, w1)
        h = _silu(h)
        out = jnp.einsum("bsf,fd->bsd", h, w2)
        return out

    x = A_x
    h = x + _A_ref(_layernorm(x, axis=-1), A_wqkv, A_wo)
    h2 = h + _B_ref(_layernorm(h, axis=-1), B_w1, B_w2)
    return h2
```

```python
import functools

import jax
import jax.numpy as jnp
from jax import lax
import jax.experimental.pallas as pl
import jax.experimental.pallas.tpu as pltpu

BF = jnp.bfloat16
F32 = jnp.float32
U32 = jnp.uint32

S, D, F = 2048, 1024, 3584
WIN, DIL, DH = 8, 2, 32
EPS = 1e-5
SCALE = DH ** -0.5
LOG2E = 1.4426950408889634

TM = 512
NB = S // TM
NCH = F // 512
HALO = 16

TUNE = dict(
    first_scores=0.6, scores=0.9, last_scores=1.0,
    mix=0.4, last_mix=0.8, first_forms=0.5, norm=0.5,
    weights=(1, 0, 0, 1, 3, 3, 0, 0, 3, 3, 0, 0, 0, 0),
    prep_lead=1.05, lead=1.05, first_lead=1.2, out_lead=1.2,
    early_products=16, send=0.85, silu_cost=14,
)


def _quad(g):
    n = len(g) // 2
    return ([r[:n] for r in g[:n]], [r[n:] for r in g[:n]],
            [r[:n] for r in g[n:]], [r[n:] for r in g[n:]])


def _add(a, b):
    return [[x + y for x, y in zip(r, s)] for r, s in zip(a, b)]


def _sub(a, b):
    return [[x - y for x, y in zip(r, s)] for r, s in zip(a, b)]


def lhs_forms(g):
    if len(g) == 1:
        yield g[0][0]
        return
    a11, a12, a21, a22 = _quad(g)
    yield from lhs_forms(_add(a11, a22))
    yield from lhs_forms(_add(a21, a22))
    yield from lhs_forms(a11)
    yield from lhs_forms(a22)
    yield from lhs_forms(_add(a11, a12))
    yield from lhs_forms(_sub(a21, a11))
    yield from lhs_forms(_sub(a12, a22))


def rhs_forms(g):
    if len(g) == 1:
        yield g[0][0]
        return
    b11, b12, b21, b22 = _quad(g)
    yield from rhs_forms(_add(b11, b22))
    yield from rhs_forms(b11)
    yield from rhs_forms(_sub(b12, b22))
    yield from rhs_forms(_sub(b21, b11))
    yield from rhs_forms(b22)
    yield from rhs_forms(_add(b11, b12))
    yield from rhs_forms(_add(b21, b22))


def out_forms(get, lo, count):
    if count == 1:
        return [[get(lo)]]
    c = count // 7
    m1 = yield from out_forms(get, lo, c)
    m2 = yield from out_forms(get, lo + c, c)
    c22 = _sub(m1, m2)
    m3 = yield from out_forms(get, lo + 2 * c, c)
    c22 = _add(c22, m3)
    m4 = yield from out_forms(get, lo + 3 * c, c)
    c21 = _add(m2, m4)
    c11 = _add(m1, m4)
    m5 = yield from out_forms(get, lo + 4 * c, c)
    c12 = _add(m3, m5)
    c11 = _sub(c11, m5)
    m6 = yield from out_forms(get, lo + 5 * c, c)
    c22 = _add(c22, m6)
    m7 = yield from out_forms(get, lo + 6 * c, c)
    c11 = _add(c11, m7)
    if count == 7:
        yield
    return [r + s for r, s in zip(c11, c12)] + [r + s for r, s in zip(c21, c22)]


def emit_forms(left, n, get, put):
    forms = lhs_forms if left else rhs_forms
    if n < 4:
        for i, f in enumerate(forms([[get(r, c) for c in range(n)] for r in range(n)])):
            put(i, f.astype(BF))
        return

    def quad(r, c):
        return [[get(2 * r + i, 2 * c + j) for j in range(2)] for i in range(2)]

    def group(g, grid):
        for i, f in enumerate(forms(grid)):
            put(7 * g + i, f.astype(BF))

    x11 = quad(0, 0)
    yield
    group(2 if left else 1, x11)
    yield
    x22 = quad(1, 1)
    yield
    group(3 if left else 4, x22)
    yield
    group(0, _add(x11, x22))
    yield
    x12 = quad(0, 1)
    yield
    group(4 if left else 5, _add(x11, x12))
    yield
    group(6 if left else 2, _sub(x12, x22))
    yield
    x21 = quad(1, 0)
    yield
    group(1 if left else 6, _add(x21, x22))
    yield
    group(5 if left else 3, _sub(x21, x11))


def form_costs(n, fetch):
    q = 4 * fetch
    return [q, 17, q, 17, 25, q, 25, 25, q, 25, 25] if n == 4 else [q + 17]


class Split:
    def __init__(self, level):
        self.n = 2 ** level
        self.p = 7 ** level
        self.sub = 4 // self.n
        self.slabs = TM // 16 // self.n

    def slab(self, g, t):
        per = 8 // self.n
        return 8 * (t // per) + per * g + t % per

    def tile(self, c, a):
        return 4 * (a // self.sub) + self.sub * c + a % self.sub

    def forms(self, rows, cols):
        return (self.p, cols // self.n // 128, rows // self.n, 128)


ONE, TWO = Split(1), Split(2)


def mm(a, b):
    return jnp.dot(pltpu.bitcast(a, BF), pltpu.bitcast(b, BF),
                   preferred_element_type=F32)


def tile(x, j):
    return x[:, 128 * j:128 * (j + 1)]


def cat(xs, axis):
    return xs[0] if len(xs) == 1 else jnp.concatenate(xs, axis=axis)


def skew(xs, step, axis):
    return [x if t == 0 else pltpu.roll(x, t * step, axis) for t, x in enumerate(xs)]


def unskew(xs, step, axis):
    n = len(xs)
    size = xs[0].shape[axis]
    field = lax.broadcasted_iota(jnp.int32, xs[0].shape, axis) // step
    zs = [xs[-i % n] for i in range(n)]
    b = 1
    while b < n:
        bit = (field & b) != 0
        zs = [jnp.where(bit, zs[(i - b) % n], zs[i]) for i in range(n)]
        b *= 2
    return [z if j == 0 else pltpu.roll(z, size - j * step, axis)
            for j, z in enumerate(zs)]


def silu(x):
    h = 0.5 * x
    return h + h * jnp.tanh(h)


def staged(gen, costs):
    def step(last):
        next(gen, None)
        if last:
            assert next(gen, "done") == "done"
    return [(functools.partial(step, k == len(costs) - 1), c)
            for k, c in enumerate(costs)]


def run(tasks):
    for fn, _ in tasks:
        fn()


def merge(*lists):
    keyed = []
    for n, lst in enumerate(lists):
        total = sum(c for _, c in lst)
        acc = 0
        for item in lst:
            keyed.append(((acc + item[1] / 2) / total, n, item))
            acc += item[1]
    keyed.sort(key=lambda e: e[:2])
    return [e[2] for e in keyed]


def diagonal(pieces):
    depth = len(pieces[0])
    return [task for n in range(len(pieces) + depth - 1)
            for task in merge(*[pieces[n - k][k] for k in range(depth)
                                if 0 <= n - k < len(pieces)])]


def overlap(first, second):
    return diagonal(list(zip(first, second)))


def split(tasks, parts):
    total = sum(c for _, c in tasks)
    out = [[] for _ in range(parts)]
    acc = 0
    for item in tasks:
        out[min(int((acc + item[1] / 2) * parts / max(total, 1)), parts - 1)].append(item)
        acc += item[1]
    return out


def cut(tasks, share):
    n = int(len(tasks) * share)
    return tasks[:n], tasks[n:]


def each(lo, hi, fn):
    def body(i, carry):
        fn(i)
        return i
    return lax.fori_loop(lo, hi, body, jnp.int32(0))


class Pace:
    def __init__(self):
        self.never = self.latest = None
        self.phase = 0

    def reset(self, index):
        self.never, self.latest = index < 0, None

    def mark(self, product):
        self.latest = product

    def __call__(self, x):
        if self.latest is None:
            return x
        n = x.shape[0] * x.dtype.itemsize // 4
        row = min(8 * int(self.phase * self.latest.shape[0] / 8), self.latest.shape[0] - n)
        other = self.latest[row:row + n]
        if x.dtype == BF:
            other = pltpu.bitcast(other, BF)
        return jnp.where(self.never, other, x)

    def interleave(self, main, side, lead=1.0):
        total = sum(c for _, c in side)
        step = total * lead / len(main)
        done = i = 0
        for k, fn in enumerate(main):
            fn()
            start = total * lead * k / len(main)
            while i < len(side) and done + side[i][1] / 2 <= start + step:
                self.phase = min(max((done - start) / max(step, 1), 0), 1)
                side[i][0]()
                done += side[i][1]
                i += 1
        run(side[i:])


def kernel(x_hbm, wqkv_hbm, wo_hbm, w1_hbm, w2_hbm, out_hbm,
           x_s, h_s, raw_s, raw1_s, wk_s, wq_s, wv_s, wo_s, w1_s, w2_s,
           q_s, k_s, v_s, p_s, o_s, t_s, pad_s,
           x_sem, raw_sem, w_sem, out_sem, a_s, b_s):
    tune = TUNE
    hold = Pace()
    interleave = hold.interleave

    def x_copy(b):
        rows = pl.ds(b * TM, TM)
        return pltpu.make_async_copy(x_hbm.at[rows], x_s.at[rows], x_sem.at[b])

    def raw_copy(m, tiles, sem, rows=pl.ds(0, 128)):
        return pltpu.make_async_copy(
            wqkv_hbm.at[pl.ds(*tiles), rows, pl.ds(D * (1, 0, 2)[m], D)],
            raw_s.at[pl.ds(8 * m + tiles[0], tiles[1]), rows], raw_sem.at[sem])

    def w1_copy(lo, hi):
        cols = (slice(None), pl.ds(512 * lo, 512 * (hi - lo)))
        return pltpu.make_async_copy(w1_hbm.at[cols], raw1_s.at[cols], w_sem.at[lo])

    def out_copy(row, rows, half, sem):
        idx = (pl.ds(row, rows), pl.ds(512 * half, 512))
        return pltpu.make_async_copy(x_s.at[idx], out_hbm.at[idx], out_sem.at[sem])

    def wait(*copies, start=()):
        def go(n):
            for k, c in enumerate(start):
                pl.when(n == k)(c.start)
            for c in copies:
                pl.when(n == len(start))(c.wait)
        hold.reset(each(0, max(len(start) + 1, 2), go))

    def rhs_square(sp, load, put):
        return [x for ka in range(sp.sub) for na in range(sp.sub) for x in staged(
            emit_forms(False, sp.n,
                       lambda r, c, ka=ka, na=na: hold(load(
                           sp.tile(r, ka), sp.tile(c, na))).astype(F32),
                       lambda i, val, ka=ka, na=na: put(i, ka, na, val)),
            form_costs(sp.n, 4))]

    def proj_square(w_s, kc, s, a, load):
        def put(i, ka, na, val):
            w_s[i, 2 * a + na, pl.ds(128 * (2 * kc + ka) + 16 * s, 16), :] = val
        return rhs_square(ONE, load, put)

    def prep_qkv(m, w_s, halves=(0, 1), slabs=range(8)):
        def permute(kc, s, r):
            w = cat([pltpu.bitcast(raw_s[8 * m + 4 * kc + r + e, pl.ds(16 * s, 16), :], U32)
                     for e in range(2)], 0)
            xs = skew([tile(w, t) for t in range(8)], 4, 1)
            yield
            xs = unskew(xs, 4, 1)
            yield
            for c, x in enumerate(xs):
                p_s[c, pl.ds(32 * s + 8 * r, 16), :] = pltpu.bitcast(x, F32)

        tasks = []
        for kc in halves:
            pieces = []
            for s in slabs:
                for a in range(2):
                    x, y, z = staged(permute(kc, s, 2 * a), [32, 52, 16])
                    pieces.append([[x], [], [], [y], [], [], [z], [], proj_square(
                        w_s, kc, s, a, lambda r, c, s=s, a=a: pltpu.bitcast(
                            p_s[4 * a + c, pl.ds(32 * s + 8 * r, 8), :], BF))])
            tasks += diagonal(pieces)
        return tasks

    def prep_wo():
        tasks = []
        for kc in range(2):
            for s in range(8):
                for a in range(2):
                    rows = []

                    def fetch(kc=kc, s=s, a=a, rows=rows):
                        hh, t2 = divmod(s, 2)
                        rows.extend(unskew(skew([pltpu.bitcast(raw_s[
                            28 + 4 * t2 + t, pl.ds(32 * hh + 16 * kc, 16),
                            pl.ds(512 * a, 512)], U32) for t in range(4)], 2, 0), 2, 0))
                    tasks.append((fetch, 70))
                    tasks += proj_square(
                        wo_s, kc, s, a,
                        lambda r, c, rows=rows: pltpu.bitcast(tile(rows[r], c), BF))
        return tasks

    def prep_w1(j):
        def square(kc, s):
            def put(i, ka, na, val):
                w1_s[j, i, 0, pl.ds(128 * kc + 16 * s, 16), :] = val
            return rhs_square(TWO, lambda r, c: raw1_s[
                pl.ds(512 * kc + 128 * r + 16 * s, 16), pl.ds(512 * j + 128 * c, 128)], put)
        return [x for kc in range(2) for s in range(8) for x in square(kc, s)]

    def prep_w2(j):
        def square(a, s):
            def put(i, ka, na, val):
                w2_s[j, i, a, pl.ds(16 * s, 16), :] = val
            return rhs_square(TWO, lambda r, c: raw_s[
                4 * j + r, pl.ds(16 * s, 16), pl.ds(512 * a + 128 * c, 128)], put)
        return [x for a in range(2) for s in range(8) for x in square(a, s)]

    def moments(load, out):
        x = [load(j) for j in range(8)]
        mean = jnp.sum(functools.reduce(jnp.add, x), axis=-1, keepdims=True) * (1.0 / D)
        yield
        x = [t - mean for t in x]
        sq = functools.reduce(jnp.add, [t * t for t in x])
        var = jnp.sum(sq, axis=-1, keepdims=True) * (1.0 / D)
        yield
        inv = lax.rsqrt(var + EPS)
        out.append(lambda j: hold(x[j]) * inv)

    def norm(sp, load, dst, first_cost):
        stats, forms = [], []
        for t in range(sp.slabs):
            rows = [[] for _ in range(sp.n)]
            stats.append(merge(*[staged(moments(
                functools.partial(load, 16 * sp.slab(g, t)), rows[g]), [first_cost, 46, 10])
                for g in range(sp.n)]))

            def put(i, val, a, t=t):
                dst[i, a, pl.ds(16 * t, 16), :] = val
            forms.append([x for a in range(8 // sp.n) for x in staged(
                emit_forms(True, sp.n,
                           lambda r, c, a=a, rows=rows: rows[r][0](sp.tile(c, a)),
                           functools.partial(put, a=a)),
                form_costs(sp.n, 4))])
        return stats, forms

    def norm1(row0, dst):
        return norm(ONE, lambda r, j: hold(
            x_s[pl.ds(row0 + r, 16), pl.ds(128 * j, 128)]).astype(F32), dst, 38)

    def norm2(row0):
        return norm(TWO, lambda r, j: hold(h_s[j, pl.ds(row0 + r, 16), :]), b_s, 30)

    def project(lhs_s, w_s, sink, halves=False, park=True):
        stages, early = [], []
        for a0 in (0, 2):
            for r in range(2):
                m = {}

                def dot(i, k, a0=a0, r=r, m=m):
                    d = mm(cat([lhs_s.bitcast(U32)[i, 2 * k + c, pl.ds(64 * r, 64), :]
                                for c in range(2)], 1),
                           cat([w_s.bitcast(U32)[i, a0 + a, pl.ds(128 * k, 128), :]
                                for a in range(2)], 1))
                    hold.mark(tile(d, 0))
                    for a in range(2):
                        n = ((a0 + a) * 7 + i) * 256 + 128 * r
                        spot = (n // S, pl.ds(n % S, 128))
                        if halves and park and k == 0:
                            h_s[spot] = tile(d, a)
                        elif halves and park:
                            m[a, i] = h_s[spot] + tile(d, a)
                        else:
                            m[a, i] = tile(d, a) if k == 0 else m[a, i] + tile(d, a)

                def post(t, a, a0=a0, r=r, m=m):
                    c = yield from out_forms(lambda i: m[a, i][16 * t:16 * t + 16], 0, 7)
                    for g in range(2):
                        for cc in range(2):
                            sink(ONE.tile(cc, a0 + a), ONE.slab(g, 8 * r + t), c[g][cc])

                posts = [x for a in range(2) for t in range(8)
                         for x in staged(post(t, a), [18, 10])]
                if halves:
                    early.append(([functools.partial(dot, i, 0) for i in range(7)], []))
                stages.append(([functools.partial(dot, i, k) for i in range(7)
                                for k in ((1,) if halves else (0, 1))], posts))
        return (early, stages) if halves else stages

    def run_stages(stages, carried, side, lead=1.0):
        idle = sum(c for _, c in side) * (lead - 1)
        side = side + [(lambda: None, idle / 8)] * 8
        for (dots, posts), part in zip(stages, split(side, len(stages))):
            interleave(dots, carried + part)
            carried = posts
        return carried

    def to_ref(ref, off):
        def sink(j, sl, val):
            ref[j, pl.ds(off + 16 * sl, 16), :] = val
        return sink

    def residual(row0):
        def sink(j, sl, val):
            rows = pl.ds(row0 + 16 * sl, 16)
            h_s[j, rows, :] = hold(x_s[rows, pl.ds(128 * j, 128)]).astype(F32) + val
        return sink

    def scores(first_block):
        lane = lax.broadcasted_iota(jnp.int32, (8, 128), 1)
        odd, high = (lane & 1) != 0, (lane & 2) != 0
        up = lambda x, b: pltpu.roll(x, b, 1)
        down = lambda x, b: pltpu.roll(x, 128 - b, 1)

        def go(r):
            acc = [None] * WIN
            for j in range(8):
                q = hold(q_s[j, pl.ds(r, 8), :])
                for w in range(WIN):
                    kw = k_s[j, pl.ds(HALO + r - DIL * w, 8), :]
                    acc[w] = q * kw if j == 0 else acc[w] + q * kw
                if j % 2:
                    yield
            xs = [(acc[w], up(acc[w], 1), acc[w + 1], down(acc[w + 1], 1))
                  for w in range(0, WIN, 2)]
            yield
            xs = [jnp.where(odd, a + ua, b + db) for a, ua, b, db in xs]
            xs = [hold(x) for x in xs]
            xs = [(x, up(x, 2), down(x, 2)) for x in xs]
            yield
            logit = [x + jnp.where(high, u, d) for x, u, d in xs]
            if first_block and r < DIL * (WIN - 1):
                row = lax.broadcasted_iota(jnp.int32, (8, 128), 0) + r
                for n, s in enumerate(logit):
                    w = jnp.where(odd, 2 * n, 2 * n + 1)
                    logit[n] = jnp.where(row >= DIL * w, s * SCALE, -1e9)
                factor = LOG2E
            else:
                factor = SCALE * LOG2E
            top = functools.reduce(jnp.maximum, logit)
            u, d = up(top, 1), down(top, 1)
            yield
            top = jnp.maximum(top, jnp.where(odd, u, d))
            e = [jnp.exp2((s - top) * factor) for s in logit]
            total = functools.reduce(jnp.add, e)
            u, d = up(total, 1), down(total, 1)
            yield
            inv = 1.0 / (total + jnp.where(odd, u, d))
            e = [x * inv for x in e]
            xs = [(x, up(x, 1), down(x, 1)) for x in e]
            yield
            e = [y for x, u, d in xs for y in (jnp.where(odd, x, d), jnp.where(odd, u, x))]
            for w in range(WIN):
                p_s[w, pl.ds(r, 8), :] = e[w]

        pieces = [staged(go(r), [32] * 4 + [8, 20, 12, 16, 16, 16]) for r in range(0, TM, 8)]
        return [task for n in range(len(pieces) + 6) for task in merge(
            pieces[n][:4] if n < len(pieces) else [],
            [pieces[n - k][3 + k] for k in range(1, 7) if 0 <= n - k < len(pieces)])]

    def mix(dst):
        def go(t, a):
            grid = [[], []]
            for g in range(2):
                r = 16 * ONE.slab(g, t)
                p = [hold(p_s[w, pl.ds(r, 16), :]) for w in range(WIN)]
                for c in range(2):
                    terms = []
                    for w in range(WIN // 2):
                        v = v_s[ONE.tile(c, a), pl.ds(HALO + r - DIL * w - 8, 24), :]
                        terms.append(p[w] * v[8:] + p[w + 4] * v[:16])
                    grid[g].append((terms[0] + terms[1]) + (terms[2] + terms[3]))
                    yield

            def put(i, val):
                dst[i, a, pl.ds(16 * t, 16), :] = val
            yield from emit_forms(True, 2, lambda g, c: grid[g][c], put)

        return [x for lo in (0, 2) for t in range(ONE.slabs) for a in (lo, lo + 1)
                for x in staged(go(t, a), [46, 30, 46, 30, 17])]

    def halo(ref):
        def keep():
            ref[:, pl.ds(0, HALO), :] = ref[:, pl.ds(TM, HALO), :]
        return [(keep, 0)]

    def first_halo():
        for j in range(8):
            v_s[j, pl.ds(0, HALO), :] = jnp.broadcast_to(
                v_s[j, pl.ds(HALO, 1), :], (HALO, 128))

    def expand():
        stages = []
        for j in range(NCH):
            m = [None] * TWO.p

            def dot(p, j=j, m=m):
                m[p] = mm(cat([b_s.bitcast(U32)[p, c] for c in range(2)], 1),
                          w1_s.bitcast(U32)[j, p, 0])
                hold.mark(m[p])

            def post(t, j=j, m=m):
                c = yield from out_forms(lambda p: m[p][16 * t:16 * t + 16], 0, TWO.p)

                def put(p, val):
                    t_s[p, j, pl.ds(16 * t, 16), :] = val
                yield from emit_forms(True, 4, lambda g, cc: silu(hold(c[g][cc])), put)

            stages.append(([functools.partial(dot, p) for p in range(TWO.p)],
                           [x for t in range(TWO.slabs) for x in staged(
                               post(t), [0] * 7 + form_costs(4, tune["silu_cost"]))]))
        return stages

    def parked(p, rows=slice(None)):
        ref, start = (q_s, p_s)[p // 32], 128 * (p % 4)
        lo, hi, _ = rows.indices(128)
        return ref, (p % 32 // 4, pl.ds(start + lo, hi - lo))

    def contract(row0, a):
        m = [None] * TWO.p

        def dot(p, j0, j1):
            d = mm(cat([t_s.bitcast(U32)[p, j] for j in range(j0, j1)], 1),
                   cat([w2_s.bitcast(U32)[j, p, a] for j in range(j0, j1)], 0))
            m[p] = d if m[p] is None else m[p] + d
            hold.mark(d)
            if a and j1 == NCH:
                ref, idx = parked(p)
                ref[idx] = m[p]

        def product(p, t):
            if not a:
                return m[p][16 * t:16 * t + 16]
            ref, idx = parked(p, slice(16 * t, 16 * t + 16))
            return hold(ref[idx])

        def post(t):
            c = yield from out_forms(lambda p: product(p, t), 0, TWO.p)
            for g in range(4):
                rows = pl.ds(row0 + 16 * TWO.slab(g, t), 16)
                x_s[rows, pl.ds(512 * a, 512)] = cat(
                    [h_s[4 * a + cc, rows, :] + (c[g][cc] if a else hold(c[g][cc]))
                     for cc in range(4)], 1).astype(BF)
                if g == 1:
                    yield

        def dots(products, *edges):
            return [functools.partial(dot, p, j0, j1) for p in products
                    for j0, j1 in zip(edges, edges[1:])]

        posts = [x for t in range(TWO.slabs)
                 for x in staged(post(t), [30 if a else 0] * 7 + [36] * 2)]
        if a:
            return [(dots(range(TWO.p), 0, 2, 4, NCH), posts)]
        n = tune["early_products"]
        return [(dots(range(n), 0, 2, 4, NCH - 1), []),
                (dots(range(n), NCH - 1, NCH) + dots(range(n, TWO.p), 0, 2, 4, NCH), posts)]

    k_stages = lambda lhs, **kw: project(lhs, wk_s, to_ref(k_s, HALO), **kw)
    q_stages = lambda lhs, **kw: project(lhs, wq_s, to_ref(q_s, 0), **kw)
    v_stages = lambda lhs: project(lhs, wv_s, to_ref(v_s, HALO))
    o_stages = lambda b, lhs, **kw: project(lhs, wo_s, residual(b * TM), **kw)
    flat = lambda parts: [x for part in parts for x in part]
    lead, prep_lead = tune["lead"], tune["prep_lead"]

    jobs = [f(j) for f in (prep_w1, prep_w2) for j in range(NCH)]
    take = lambda n: flat([jobs.pop(0) for _ in range(n)])
    first_stats, first_forms = (flat(x) for x in norm2(0))

    head = [raw_copy(0, (0, 4), h, pl.ds(64 * h, 64)) for h in range(2)]
    k1, q0, q1, v = (raw_copy(0, (4, 4), 2), raw_copy(1, (0, 4), 3),
                     raw_copy(1, (4, 4), 4), raw_copy(2, (0, 8), 5))
    wo = pltpu.make_async_copy(wo_hbm, raw_s.at[pl.ds(28, 8)], raw_sem.at[6])
    w1 = [w1_copy(0, 1), w1_copy(1, 2), w1_copy(2, NCH)]
    w2 = pltpu.make_async_copy(w2_hbm, raw_s.at[pl.ds(0, 28)], w_sem.at[3])
    fence = pltpu.make_async_copy(wo_hbm.at[0, pl.ds(0, 16)], pad_s, raw_sem.at[7])

    wait(x_copy(0), start=[x_copy(0), *head, k1, q0, q1, x_copy(1), v, wo, x_copy(2), w1[0]])
    k_s[:, pl.ds(0, HALO), :] = jnp.zeros((8, HALO, 128), F32)
    run(overlap(*norm1(0, o_s)))
    for h in range(2):
        wait(head[h])
        run(prep_qkv(0, wk_s, (0,), range(4 * h, 4 * h + 4)))
    early, late = k_stages(o_s, halves=True)
    run_stages(early[:2], [], [])
    wait(k1)
    run_stages(early[2:], [], prep_qkv(0, wk_s, (1,)), prep_lead)
    wait(q0)
    left = run_stages(late, [], prep_qkv(1, wq_s, (0,)), prep_lead)
    wait(q1, x_copy(1))
    early, late = q_stages(o_s, halves=True)
    stats, forms = (flat(x) for x in norm1(TM, a_s))
    run_stages(early, left, merge(prep_qkv(1, wq_s, (1,)), stats), prep_lead)
    wait(v)
    left = run_stages(late, [], prep_qkv(2, wv_s), prep_lead)
    wait(start=[w1[1]])
    sc_a, sc_b = cut(scores(True), tune["first_scores"])
    left = run_stages(v_stages(o_s), left, merge(sc_a, forms), tune["first_lead"])

    for b in range(1, NB):
        last = b == NB - 1
        nk, nq, nv, no = tune["weights"][4 * b - 4:4 * b]
        mix_a, mix_b = cut(mix(o_s), 0.0 if b == 1 else tune["mix"])
        if b == 1:
            wait(wo, x_copy(2), w1[0], start=[w1[2], w2, x_copy(3), fence])
            stages = k_stages(a_s)
            interleave(flat(st[0] for st in stages[:2]), merge(left, sc_b), lead=1.1)
            left = [(first_halo, 0)] + halo(k_s) + flat(st[1] for st in stages[:2])
            left = run_stages(stages[2:], left, prep_wo() + take(nk))
        else:
            left = run_stages(k_stages(a_s), halo(k_s) + left, merge(mix_a, take(nk)))
        if b == 2:
            wait(w2, x_copy(3))
        left = run_stages(q_stages(a_s), left, merge(mix_b, take(nq)), lead)
        if b == 1:
            wait(w1[1], w1[2])
        if last:
            wait(fence)
        sc_a, sc_b = cut(scores(False), tune["last_scores" if last else "scores"])
        stats, forms = ([], []) if last else (flat(x) for x in norm1((b + 1) * TM, a_s))
        left = run_stages(v_stages(a_s), halo(v_s) + left, merge(sc_a, stats, take(nv)))
        if not last:
            left = run_stages(o_stages(b - 1, o_s), left, merge(
                sc_b, forms, first_stats if b == 2 else [], take(no)), lead)
    mix_a, mix_b = cut(mix(a_s), tune["last_mix"])
    forms_a, forms_b = cut(first_forms, tune["first_forms"])
    left = run_stages(o_stages(NB - 2, o_s), left,
                      merge(sc_b + merge(mix_a, forms_a), take(no)), lead)
    early, late = o_stages(NB - 1, a_s, halves=True, park=False)
    run_stages(early, left, merge(mix_b, forms_b, take(tune["weights"][-2])), lead)
    run(run_stages(late, [], take(tune["weights"][-1]), lead))
    assert not jobs

    def ffn_step(i, carry):
        row0 = pl.multiple_of(i * TM, TM)
        nxt = pl.multiple_of(jnp.minimum(i + 1, NB - 1) * TM, TM)
        prev = pl.multiple_of((i + NB - 1) % NB * TM, TM)
        hold.reset(i)
        left = run_stages(expand(), contract(prev, 1)[0][1], [])
        one, two = contract(row0, 0)
        interleave(one[0], left)
        norm_a, norm_b = cut(overlap(*norm2(nxt)), tune["norm"])
        left = run_stages([two], [], norm_a)
        dots = contract(row0, 1)[0][0]
        n = int(len(dots) * tune["send"]) // 3 * 3
        interleave(dots[:n], merge(left, norm_b), lead=tune["out_lead"])

        def send(k):
            pl.when(k == 1)(out_copy(row0, TM, 0, 2 * i).start)
            pl.when(k == 0)(out_copy(prev, TM, 1, jnp.maximum(2 * i - 1, 0)).start)
        each(jnp.where(i > 0, 0, 1), 2, send)
        run([(d, 0) for d in dots[n:]])
        return carry

    lax.fori_loop(0, NB, ffn_step, 0)
    hold.latest = None
    tail = [out_copy(S - TM + 128 * u, 128, 1, 2 * NB - 1 + u) for u in range(4)]
    for tasks, c in zip(split(contract(S - TM, 1)[0][1], 4), tail):
        run(tasks)
        c.start()
    for c in [out_copy(n // 2 * TM, TM, n % 2, n) for n in range(2 * NB - 1)] + tail:
        c.wait()


@jax.jit
def pallas_sequential_preLN__sliding_local_dilated__dense_activation_silu__prompt_kernel(
    A_x: jax.Array,
    A_wqkv: jax.Array,
    A_wo: jax.Array,
    B_x: jax.Array,
    B_w1: jax.Array,
    B_w2: jax.Array,
):
    del B_x
    scratch = [
        pltpu.VMEM((S, D), BF),
        pltpu.VMEM((8, S, 128), F32),
        pltpu.VMEM((36, 128, D), BF),
        pltpu.VMEM((D, F), BF),
        pltpu.VMEM(ONE.forms(D, D), BF),
        pltpu.VMEM(ONE.forms(D, D), BF),
        pltpu.VMEM(ONE.forms(D, D), BF),
        pltpu.VMEM(ONE.forms(D, D), BF),
        pltpu.VMEM((NCH,) + TWO.forms(D, 512), BF),
        pltpu.VMEM((NCH,) + TWO.forms(512, D), BF),
        pltpu.VMEM((8, TM, 128), F32),
        pltpu.VMEM((8, HALO + TM, 128), F32),
        pltpu.VMEM((8, HALO + TM, 128), F32),
        pltpu.VMEM((WIN, TM, 128), F32),
        pltpu.VMEM(ONE.forms(TM, D), BF),
        pltpu.VMEM(TWO.forms(TM, F), BF),
        pltpu.VMEM((16, D), BF),
        pltpu.SemaphoreType.DMA((NB,)),
        pltpu.SemaphoreType.DMA((8,)),
        pltpu.SemaphoreType.DMA((4,)),
        pltpu.SemaphoreType.DMA((2 * NB + 3,)),
        pltpu.VMEM(ONE.forms(TM, D), BF),
        pltpu.VMEM(TWO.forms(TM, D), BF),
    ]
    out = pl.pallas_call(
        kernel,
        in_specs=[pl.BlockSpec(memory_space=pl.ANY)] * 5,
        out_specs=pl.BlockSpec(memory_space=pl.ANY),
        out_shape=jax.ShapeDtypeStruct((S, D), BF),
        scratch_shapes=scratch,
        compiler_params=pltpu.CompilerParams(vmem_limit_bytes=126 << 20),
    )(A_x.reshape(S, D), A_wqkv.reshape(8, 128, 3 * D), A_wo.reshape(8, 128, D),
      B_w1, B_w2.reshape(F // 128, 128, D))
    return out.reshape(1, S, D)
```

```python
import functools

import jax
import jax.numpy as jnp
from jax import lax
import jax.experimental.pallas as pl
import jax.experimental.pallas.tpu as pltpu

BF = jnp.bfloat16
F32 = jnp.float32
U32 = jnp.uint32

S, D, F = 2048, 1024, 3584
WIN, DIL, DH = 8, 2, 32
EPS = 1e-5
SCALE = DH ** -0.5
LOG2E = 1.4426950408889634

TM = 512
NB = S // TM
NCH = F // 512
HALO = 16

TUNE = dict(
    first_scores=0.4, scores=0.9, last_scores=1.0,
    mix=0.55, last_mix=0.8, early_forms=0.4, first_forms=0.5, norm=0.6,
    weights=(1, 0, 0, 1, 2, 3, 0, 0, 2, 3, 0, 0, 1, 1),
    prep_lead=1.05, lead=1.05, first_lead=1.2, out_lead=1.2,
    early_products=16, send=0.85, silu_cost=14,
)


def _quad(g):
    n = len(g) // 2
    return ([r[:n] for r in g[:n]], [r[n:] for r in g[:n]],
            [r[:n] for r in g[n:]], [r[n:] for r in g[n:]])


def _add(a, b):
    return [[x + y for x, y in zip(r, s)] for r, s in zip(a, b)]


def _sub(a, b):
    return [[x - y for x, y in zip(r, s)] for r, s in zip(a, b)]


def lhs_forms(g):
    if len(g) == 1:
        yield g[0][0]
        return
    a11, a12, a21, a22 = _quad(g)
    yield from lhs_forms(_add(a11, a22))
    yield from lhs_forms(_add(a21, a22))
    yield from lhs_forms(a11)
    yield from lhs_forms(a22)
    yield from lhs_forms(_add(a11, a12))
    yield from lhs_forms(_sub(a21, a11))
    yield from lhs_forms(_sub(a12, a22))


def rhs_forms(g):
    if len(g) == 1:
        yield g[0][0]
        return
    b11, b12, b21, b22 = _quad(g)
    yield from rhs_forms(_add(b11, b22))
    yield from rhs_forms(b11)
    yield from rhs_forms(_sub(b12, b22))
    yield from rhs_forms(_sub(b21, b11))
    yield from rhs_forms(b22)
    yield from rhs_forms(_add(b11, b12))
    yield from rhs_forms(_add(b21, b22))


def out_forms(get, lo, count):
    if count == 1:
        return [[get(lo)]]
    c = count // 7
    m1 = yield from out_forms(get, lo, c)
    m2 = yield from out_forms(get, lo + c, c)
    c22 = _sub(m1, m2)
    m3 = yield from out_forms(get, lo + 2 * c, c)
    c22 = _add(c22, m3)
    m4 = yield from out_forms(get, lo + 3 * c, c)
    c21 = _add(m2, m4)
    c11 = _add(m1, m4)
    m5 = yield from out_forms(get, lo + 4 * c, c)
    c12 = _add(m3, m5)
    c11 = _sub(c11, m5)
    m6 = yield from out_forms(get, lo + 5 * c, c)
    c22 = _add(c22, m6)
    m7 = yield from out_forms(get, lo + 6 * c, c)
    c11 = _add(c11, m7)
    if count == 7:
        yield
    return [r + s for r, s in zip(c11, c12)] + [r + s for r, s in zip(c21, c22)]


def emit_forms(left, n, get, put):
    forms = lhs_forms if left else rhs_forms
    if n < 4:
        for i, f in enumerate(forms([[get(r, c) for c in range(n)] for r in range(n)])):
            put(i, f.astype(BF))
        return

    def quad(r, c):
        return [[get(2 * r + i, 2 * c + j) for j in range(2)] for i in range(2)]

    def group(g, grid):
        for i, f in enumerate(forms(grid)):
            put(7 * g + i, f.astype(BF))

    x11 = quad(0, 0)
    yield
    group(2 if left else 1, x11)
    yield
    x22 = quad(1, 1)
    yield
    group(3 if left else 4, x22)
    yield
    group(0, _add(x11, x22))
    yield
    x12 = quad(0, 1)
    yield
    group(4 if left else 5, _add(x11, x12))
    yield
    group(6 if left else 2, _sub(x12, x22))
    yield
    x21 = quad(1, 0)
    yield
    group(1 if left else 6, _add(x21, x22))
    yield
    group(5 if left else 3, _sub(x21, x11))


def form_costs(n, fetch):
    q = 4 * fetch
    return [q, 17, q, 17, 25, q, 25, 25, q, 25, 25] if n == 4 else [q + 17]


class Split:
    def __init__(self, level):
        self.n = 2 ** level
        self.p = 7 ** level
        self.sub = 4 // self.n
        self.slabs = TM // 16 // self.n

    def slab(self, g, t):
        per = 8 // self.n
        return 8 * (t // per) + per * g + t % per

    def tile(self, c, a):
        return 4 * (a // self.sub) + self.sub * c + a % self.sub

    def forms(self, rows, cols):
        return (self.p, cols // self.n // 128, rows // self.n, 128)


ONE, TWO = Split(1), Split(2)


def mm(a, b):
    return jnp.dot(pltpu.bitcast(a, BF), pltpu.bitcast(b, BF),
                   preferred_element_type=F32)


def tile(x, j):
    return x[:, 128 * j:128 * (j + 1)]


def cat(xs, axis):
    return xs[0] if len(xs) == 1 else jnp.concatenate(xs, axis=axis)


def skew(xs, step, axis):
    return [x if t == 0 else pltpu.roll(x, t * step, axis) for t, x in enumerate(xs)]


def unskew(xs, step, axis):
    n = len(xs)
    size = xs[0].shape[axis]
    field = lax.broadcasted_iota(jnp.int32, xs[0].shape, axis) // step
    zs = [xs[-i % n] for i in range(n)]
    b = 1
    while b < n:
        bit = (field & b) != 0
        zs = [jnp.where(bit, zs[(i - b) % n], zs[i]) for i in range(n)]
        b *= 2
    return [z if j == 0 else pltpu.roll(z, size - j * step, axis)
            for j, z in enumerate(zs)]


def silu(x):
    h = 0.5 * x
    return h + h * jnp.tanh(h)


def staged(gen, costs):
    def step(last):
        next(gen, None)
        if last:
            assert next(gen, "done") == "done"
    return [(functools.partial(step, k == len(costs) - 1), c)
            for k, c in enumerate(costs)]


def run(tasks):
    for fn, _ in tasks:
        fn()


def merge(*lists):
    keyed = []
    for n, lst in enumerate(lists):
        total = sum(c for _, c in lst)
        acc = 0
        for item in lst:
            keyed.append(((acc + item[1] / 2) / total, n, item))
            acc += item[1]
    keyed.sort(key=lambda e: e[:2])
    return [e[2] for e in keyed]


def diagonal(pieces):
    depth = len(pieces[0])
    return [task for n in range(len(pieces) + depth - 1)
            for task in merge(*[pieces[n - k][k] for k in range(depth)
                                if 0 <= n - k < len(pieces)])]


def overlap(first, second):
    return diagonal(list(zip(first, second)))


def split(tasks, parts):
    total = sum(c for _, c in tasks)
    out = [[] for _ in range(parts)]
    acc = 0
    for item in tasks:
        out[min(int((acc + item[1] / 2) * parts / max(total, 1)), parts - 1)].append(item)
        acc += item[1]
    return out


def cut(tasks, share):
    n = int(len(tasks) * share)
    return tasks[:n], tasks[n:]


def each(lo, hi, fn):
    def body(i, carry):
        fn(i)
        return i
    return lax.fori_loop(lo, hi, body, jnp.int32(0))


class Pace:
    def __init__(self):
        self.never = self.latest = None
        self.phase = 0

    def reset(self, index):
        self.never, self.latest = index < 0, None

    def mark(self, product):
        self.latest = product

    def __call__(self, x):
        if self.latest is None:
            return x
        n = x.shape[0] * x.dtype.itemsize // 4
        row = min(8 * int(self.phase * self.latest.shape[0] / 8), self.latest.shape[0] - n)
        other = self.latest[row:row + n]
        if x.dtype == BF:
            other = pltpu.bitcast(other, BF)
        return jnp.where(self.never, other, x)

    def interleave(self, main, side, lead=1.0):
        total = sum(c for _, c in side)
        step = total * lead / len(main)
        done = i = 0
        for k, fn in enumerate(main):
            fn()
            start = total * lead * k / len(main)
            while i < len(side) and done + side[i][1] / 2 <= start + step:
                self.phase = min(max((done - start) / max(step, 1), 0), 1)
                side[i][0]()
                done += side[i][1]
                i += 1
        run(side[i:])


def kernel(x_hbm, wqkv_hbm, wo_hbm, w1_hbm, w2_hbm, out_hbm,
           x_s, h_s, raw_s, raw1_s, wk_s, wq_s, wv_s, wo_s, w1_s, w2_s,
           q_s, k_s, v_s, p_s, o_s, t_s, pad_s,
           x_sem, raw_sem, w_sem, out_sem, a_s, b_s):
    tune = TUNE
    hold = Pace()
    interleave = hold.interleave

    def x_copy(b):
        rows = pl.ds(b * TM, TM)
        return pltpu.make_async_copy(x_hbm.at[rows], x_s.at[rows], x_sem.at[b])

    def raw_copy(m, tiles, sem, rows=slice(None)):
        return pltpu.make_async_copy(
            wqkv_hbm.at[pl.ds(*tiles), rows, pl.ds(D * (1, 0, 2)[m], D)],
            raw_s.at[pl.ds(8 * m + tiles[0], tiles[1]), rows], raw_sem.at[sem])

    def w1_copy(lo, hi):
        cols = (slice(None), pl.ds(512 * lo, 512 * (hi - lo)))
        return pltpu.make_async_copy(w1_hbm.at[cols], raw1_s.at[cols], w_sem.at[lo])

    def out_copy(row, rows, half, sem):
        idx = (pl.ds(row, rows), pl.ds(512 * half, 512))
        return pltpu.make_async_copy(x_s.at[idx], out_hbm.at[idx], out_sem.at[sem])

    def wait(*copies, start=()):
        def go(n):
            for k, c in enumerate(start):
                pl.when(n == k)(c.start)
            for c in copies:
                pl.when(n == len(start))(c.wait)
        hold.reset(each(0, max(len(start) + 1, 2), go))

    def rhs_square(sp, load, put):
        return [x for ka in range(sp.sub) for na in range(sp.sub) for x in staged(
            emit_forms(False, sp.n,
                       lambda r, c, ka=ka, na=na: hold(load(
                           sp.tile(r, ka), sp.tile(c, na))).astype(F32),
                       lambda i, val, ka=ka, na=na: put(i, ka, na, val)),
            form_costs(sp.n, 4))]

    def proj_square(w_s, kc, s, a, load):
        def put(i, ka, na, val):
            w_s[i, 2 * a + na, pl.ds(128 * (2 * kc + ka) + 16 * s, 16), :] = val
        return rhs_square(ONE, load, put)

    def prep_qkv(m, w_s, halves=(0, 1), slabs=range(8)):
        def permute(kc, s, r):
            w = cat([pltpu.bitcast(raw_s[8 * m + 4 * kc + r + e, pl.ds(16 * s, 16), :], U32)
                     for e in range(2)], 0)
            xs = skew([tile(w, t) for t in range(8)], 4, 1)
            yield
            xs = unskew(xs, 4, 1)
            yield
            for c, x in enumerate(xs):
                p_s[c, pl.ds(256 * kc + 32 * s + 8 * r, 16), :] = pltpu.bitcast(x, F32)

        tasks = []
        for kc in halves:
            pieces = []
            for s in slabs:
                for a in range(2):
                    x, y, z = staged(permute(kc, s, 2 * a), [32, 52, 16])
                    pieces.append([[x], [], [], [y], [], [], [z], [], proj_square(
                        w_s, kc, s, a, lambda r, c, s=s, a=a, kc=kc: pltpu.bitcast(
                            p_s[4 * a + c, pl.ds(256 * kc + 32 * s + 8 * r, 8), :], BF))])
            tasks += diagonal(pieces)
        return tasks

    def prep_wo():
        tasks = []
        for kc in range(2):
            for s in range(8):
                for a in range(2):
                    rows = []

                    def fetch(kc=kc, s=s, a=a, rows=rows):
                        hh, t2 = divmod(s, 2)
                        rows.extend(unskew(skew([pltpu.bitcast(raw_s[
                            28 + 4 * t2 + t, pl.ds(32 * hh + 16 * kc, 16),
                            pl.ds(512 * a, 512)], U32) for t in range(4)], 2, 0), 2, 0))
                    tasks.append((fetch, 70))
                    tasks += proj_square(
                        wo_s, kc, s, a,
                        lambda r, c, rows=rows: pltpu.bitcast(tile(rows[r], c), BF))
        return tasks

    def prep_w1(j):
        def square(kc, s):
            def put(i, ka, na, val):
                w1_s[j, i, 0, pl.ds(128 * kc + 16 * s, 16), :] = val
            return rhs_square(TWO, lambda r, c: raw1_s[
                pl.ds(512 * kc + 128 * r + 16 * s, 16), pl.ds(512 * j + 128 * c, 128)], put)
        return [x for kc in range(2) for s in range(8) for x in square(kc, s)]

    def prep_w2(j):
        def square(a, s):
            def put(i, ka, na, val):
                w2_s[j, i, a, pl.ds(16 * s, 16), :] = val
            return rhs_square(TWO, lambda r, c: raw_s[
                4 * j + r, pl.ds(16 * s, 16), pl.ds(512 * a + 128 * c, 128)], put)
        return [x for a in range(2) for s in range(8) for x in square(a, s)]

    def moments(load, out):
        x = [load(j) for j in range(8)]
        mean = jnp.sum(functools.reduce(jnp.add, x), axis=-1, keepdims=True) * (1.0 / D)
        yield
        x = [t - mean for t in x]
        sq = functools.reduce(jnp.add, [t * t for t in x])
        var = jnp.sum(sq, axis=-1, keepdims=True) * (1.0 / D)
        yield
        inv = lax.rsqrt(var + EPS)
        out.append(lambda j: hold(x[j]) * inv)

    def norm(sp, load, dst, first_cost):
        stats, forms = [], []
        for t in range(sp.slabs):
            rows = [[] for _ in range(sp.n)]
            stats.append(merge(*[staged(moments(
                functools.partial(load, 16 * sp.slab(g, t)), rows[g]), [first_cost, 46, 10])
                for g in range(sp.n)]))

            def put(i, val, a, t=t):
                dst[i, a, pl.ds(16 * t, 16), :] = val
            forms.append([x for a in range(8 // sp.n) for x in staged(
                emit_forms(True, sp.n,
                           lambda r, c, a=a, rows=rows: rows[r][0](sp.tile(c, a)),
                           functools.partial(put, a=a)),
                form_costs(sp.n, 4))])
        return stats, forms

    def norm1(row0, dst):
        return norm(ONE, lambda r, j: hold(
            x_s[pl.ds(row0 + r, 16), pl.ds(128 * j, 128)]).astype(F32), dst, 38)

    def norm2(row0):
        return norm(TWO, lambda r, j: hold(h_s[j, pl.ds(row0 + r, 16), :]), b_s, 30)

    def project(lhs_s, w_s, sink, halves=False, park=True):
        stages, early = [], []
        for a0 in (0, 2):
            for r in range(2):
                m = {}

                def dot(i, k, a0=a0, r=r, m=m):
                    d = mm(cat([lhs_s.bitcast(U32)[i, 2 * k + c, pl.ds(64 * r, 64), :]
                                for c in range(2)], 1),
                           cat([w_s.bitcast(U32)[i, a0 + a, pl.ds(128 * k, 128), :]
                                for a in range(2)], 1))
                    hold.mark(tile(d, 0))
                    for a in range(2):
                        n = ((a0 + a) * 7 + i) * 256 + 128 * r
                        spot = (n // S, pl.ds(n % S, 128))
                        if halves and park and k == 0:
                            h_s[spot] = tile(d, a)
                        elif halves and park:
                            m[a, i] = h_s[spot] + tile(d, a)
                        else:
                            m[a, i] = tile(d, a) if k == 0 else m[a, i] + tile(d, a)

                def post(t, a, a0=a0, r=r, m=m):
                    c = yield from out_forms(lambda i: m[a, i][16 * t:16 * t + 16], 0, 7)
                    for g in range(2):
                        for cc in range(2):
                            sink(ONE.tile(cc, a0 + a), ONE.slab(g, 8 * r + t), c[g][cc])

                posts = [x for a in range(2) for t in range(8)
                         for x in staged(post(t, a), [18, 10])]
                if halves:
                    early.append(([functools.partial(dot, i, 0) for i in range(7)], []))
                stages.append(([functools.partial(dot, i, k) for i in range(7)
                                for k in ((1,) if halves else (0, 1))], posts))
        return (early, stages) if halves else stages

    def run_stages(stages, carried, side, lead=1.0):
        idle = sum(c for _, c in side) * (lead - 1)
        side = side + [(lambda: None, idle / 8)] * 8
        for (dots, posts), part in zip(stages, split(side, len(stages))):
            interleave(dots, carried + part)
            carried = posts
        return carried

    def to_ref(ref, off):
        def sink(j, sl, val):
            ref[j, pl.ds(off + 16 * sl, 16), :] = val
        return sink

    def residual(row0):
        def sink(j, sl, val):
            rows = pl.ds(row0 + 16 * sl, 16)
            h_s[j, rows, :] = hold(x_s[rows, pl.ds(128 * j, 128)]).astype(F32) + val
        return sink

    def scores(first_block):
        lane = lax.broadcasted_iota(jnp.int32, (8, 128), 1)
        odd, high = (lane & 1) != 0, (lane & 2) != 0
        up = lambda x, b: pltpu.roll(x, b, 1)
        down = lambda x, b: pltpu.roll(x, 128 - b, 1)

        def go(r):
            acc = [None] * WIN
            for j in range(8):
                q = hold(q_s[j, pl.ds(r, 8), :])
                for w in range(WIN):
                    kw = k_s[j, pl.ds(HALO + r - DIL * w, 8), :]
                    acc[w] = q * kw if j == 0 else acc[w] + q * kw
                if j % 2:
                    yield
            xs = [(acc[w], up(acc[w], 1), acc[w + 1], down(acc[w + 1], 1))
                  for w in range(0, WIN, 2)]
            yield
            xs = [jnp.where(odd, a + ua, b + db) for a, ua, b, db in xs]
            xs = [hold(x) for x in xs]
            xs = [(x, up(x, 2), down(x, 2)) for x in xs]
            yield
            logit = [x + jnp.where(high, u, d) for x, u, d in xs]
            if first_block and r < DIL * (WIN - 1):
                row = lax.broadcasted_iota(jnp.int32, (8, 128), 0) + r
                for n, s in enumerate(logit):
                    w = jnp.where(odd, 2 * n, 2 * n + 1)
                    logit[n] = jnp.where(row >= DIL * w, s * SCALE, -1e9)
                factor = LOG2E
            else:
                factor = SCALE * LOG2E
            top = functools.reduce(jnp.maximum, logit)
            u, d = up(top, 1), down(top, 1)
            yield
            top = jnp.maximum(top, jnp.where(odd, u, d))
            e = [jnp.exp2((s - top) * factor) for s in logit]
            total = functools.reduce(jnp.add, e)
            u, d = up(total, 1), down(total, 1)
            yield
            inv = 1.0 / (total + jnp.where(odd, u, d))
            e = [x * inv for x in e]
            xs = [(x, up(x, 1), down(x, 1)) for x in e]
            yield
            e = [y for x, u, d in xs for y in (jnp.where(odd, x, d), jnp.where(odd, u, x))]
            for w in range(WIN):
                p_s[w, pl.ds(r, 8), :] = e[w]

        pieces = [staged(go(r), [32] * 4 + [8, 20, 12, 16, 16, 16]) for r in range(0, TM, 8)]
        return [task for n in range(len(pieces) + 6) for task in merge(
            pieces[n][:4] if n < len(pieces) else [],
            [pieces[n - k][3 + k] for k in range(1, 7) if 0 <= n - k < len(pieces)])]

    def mix(dst):
        def go(t, a):
            grid = [[], []]
            for g in range(2):
                r = 16 * ONE.slab(g, t)
                p = [hold(p_s[w, pl.ds(r, 16), :]) for w in range(WIN)]
                for c in range(2):
                    terms = []
                    for w in range(WIN // 2):
                        v = v_s[ONE.tile(c, a), pl.ds(HALO + r - DIL * w - 8, 24), :]
                        terms.append(p[w] * v[8:] + p[w + 4] * v[:16])
                    grid[g].append((terms[0] + terms[1]) + (terms[2] + terms[3]))
                    yield

            def put(i, val):
                dst[i, a, pl.ds(16 * t, 16), :] = val
            yield from emit_forms(True, 2, lambda g, c: grid[g][c], put)

        return [x for lo in (0, 2) for t in range(ONE.slabs) for a in (lo, lo + 1)
                for x in staged(go(t, a), [46, 30, 46, 30, 17])]

    def halo(ref):
        def keep():
            ref[:, pl.ds(0, HALO), :] = ref[:, pl.ds(TM, HALO), :]
        return [(keep, 0)]

    def first_halo():
        for j in range(8):
            v_s[j, pl.ds(0, HALO), :] = jnp.broadcast_to(
                v_s[j, pl.ds(HALO, 1), :], (HALO, 128))

    def expand():
        stages = []
        for j in range(NCH):
            m = [None] * TWO.p

            def dot(p, j=j, m=m):
                m[p] = mm(cat([b_s.bitcast(U32)[p, c] for c in range(2)], 1),
                          w1_s.bitcast(U32)[j, p, 0])
                hold.mark(m[p])

            def post(t, j=j, m=m):
                c = yield from out_forms(lambda p: m[p][16 * t:16 * t + 16], 0, TWO.p)

                def put(p, val):
                    t_s[p, j, pl.ds(16 * t, 16), :] = val
                yield from emit_forms(True, 4, lambda g, cc: silu(hold(c[g][cc])), put)

            stages.append(([functools.partial(dot, p) for p in range(TWO.p)],
                           [x for t in range(TWO.slabs) for x in staged(
                               post(t), [0] * 7 + form_costs(4, tune["silu_cost"]))]))
        return stages

    def parked(p, rows=slice(None)):
        ref, start = (q_s, p_s)[p // 32], 128 * (p % 4)
        lo, hi, _ = rows.indices(128)
        return ref, (p % 32 // 4, pl.ds(start + lo, hi - lo))

    def contract(row0, a):
        m = [None] * TWO.p

        def dot(p, j0, j1):
            d = mm(cat([t_s.bitcast(U32)[p, j] for j in range(j0, j1)], 1),
                   cat([w2_s.bitcast(U32)[j, p, a] for j in range(j0, j1)], 0))
            m[p] = d if m[p] is None else m[p] + d
            hold.mark(d)
            if a and j1 == NCH:
                ref, idx = parked(p)
                ref[idx] = m[p]

        def product(p, t):
            if not a:
                return m[p][16 * t:16 * t + 16]
            ref, idx = parked(p, slice(16 * t, 16 * t + 16))
            return hold(ref[idx])

        def post(t):
            c = yield from out_forms(lambda p: product(p, t), 0, TWO.p)
            for g in range(4):
                rows = pl.ds(row0 + 16 * TWO.slab(g, t), 16)
                x_s[rows, pl.ds(512 * a, 512)] = cat(
                    [h_s[4 * a + cc, rows, :] + (c[g][cc] if a else hold(c[g][cc]))
                     for cc in range(4)], 1).astype(BF)
                if g == 1:
                    yield

        def dots(products, *edges):
            return [functools.partial(dot, p, j0, j1) for p in products
                    for j0, j1 in zip(edges, edges[1:])]

        posts = [x for t in range(TWO.slabs)
                 for x in staged(post(t), [30 if a else 0] * 7 + [36] * 2)]
        if a:
            return [(dots(range(TWO.p), 0, 2, 4, NCH), posts)]
        n = tune["early_products"]
        return [(dots(range(n), 0, 2, 4, NCH - 1), []),
                (dots(range(n), NCH - 1, NCH) + dots(range(n, TWO.p), 0, 2, 4, NCH), posts)]

    k_stages = lambda lhs, **kw: project(lhs, wk_s, to_ref(k_s, HALO), **kw)
    q_stages = lambda lhs, **kw: project(lhs, wq_s, to_ref(q_s, 0), **kw)
    v_stages = lambda lhs: project(lhs, wv_s, to_ref(v_s, HALO))
    o_stages = lambda b, lhs, **kw: project(lhs, wo_s, residual(b * TM), **kw)
    flat = lambda parts: [x for part in parts for x in part]
    lead, prep_lead = tune["lead"], tune["prep_lead"]

    jobs = [f(j) for f in (prep_w1, prep_w2) for j in range(NCH)]
    take = lambda n: flat([jobs.pop(0) for _ in range(n)])
    first_stats, first_forms = (flat(x) for x in norm2(0))

    head = [raw_copy(0, (0, 4), h, pl.ds(64 * h, 64)) for h in range(2)]
    k1, q0, q1, v0, v1 = (raw_copy(m, (4 * kc, 4), 2 * m + kc + 1)
                          for m, kc in ((0, 1), (1, 0), (1, 1), (2, 0), (2, 1)))
    x0 = [pltpu.make_async_copy(x_hbm.at[pl.ds(256 * r, 256)], x_s.at[pl.ds(256 * r, 256)],
                                x_sem.at[NB * r]) for r in range(2)]
    wo = pltpu.make_async_copy(wo_hbm, raw_s.at[pl.ds(28, 8)], raw_sem.at[7])
    w1 = [w1_copy(0, 1), w1_copy(1, 2), w1_copy(2, NCH)]
    w2 = pltpu.make_async_copy(w2_hbm, raw_s.at[pl.ds(0, 28)], w_sem.at[3])
    fence = pltpu.make_async_copy(wo_hbm.at[0, pl.ds(0, 16)], pad_s, raw_sem.at[8])

    wait(x0[0], start=[x0[0], head[0], x0[1], head[1], k1, q0, q1, v0, x_copy(1), v1,
                       wo, x_copy(2), w1[0]])
    k_s[:, pl.ds(0, HALO), :] = jnp.zeros((8, HALO, 128), F32)
    stats, forms = norm1(0, o_s)
    for h in range(2):
        if h:
            wait(x0[h])
        run(overlap(stats[8 * h:8 * h + 8], forms[8 * h:8 * h + 8]))
        wait(head[h])
        run(prep_qkv(0, wk_s, (0,), range(4 * h, 4 * h + 4)))
    early, late = k_stages(o_s, halves=True)
    run_stages(early[:2], [], [])
    wait(k1)
    run_stages(early[2:], [], prep_qkv(0, wk_s, (1,)), prep_lead)
    run([(d, 0) for st in late[:1] for d in st[0]])
    q0.wait()
    left = run_stages(late[1:], flat(st[1] for st in late[:1]), prep_qkv(1, wq_s, (0,)), prep_lead)
    wait(q1)
    early, late = q_stages(o_s, halves=True)
    run_stages(early, left, prep_qkv(1, wq_s, (1,)), prep_lead)
    wait(v0, x_copy(1))
    stats, forms = (flat(x) for x in norm1(TM, a_s))
    left = run_stages(late, [], merge(prep_qkv(2, wv_s, (0,)), stats), prep_lead)
    wait(v1, start=[w1[1], w1[2]])
    early, late = project(o_s, wv_s, to_ref(v_s, HALO), halves=True, park=False)
    sc_a, sc_b = cut(scores(True), tune["first_scores"])
    forms_a, forms_b = cut(forms, tune["early_forms"])
    run_stages(early, left, merge(prep_qkv(2, wv_s, (1,)), forms_a), prep_lead)
    left = run_stages(late, [], merge(sc_a, forms_b), tune["first_lead"])

    for b in range(1, NB):
        last = b == NB - 1
        nk, nq, nv, no = tune["weights"][4 * b - 4:4 * b]
        mix_a, mix_b = cut(mix(o_s), 0.0 if b == 1 else tune["mix"])
        if b == 1:
            wait(wo, x_copy(2), w1[0], start=[w2, x_copy(3), fence])
            stages = k_stages(a_s)
            interleave(flat(st[0] for st in stages[:2]), merge(left, sc_b), lead=1.1)
            left = [(first_halo, 0)] + halo(k_s) + flat(st[1] for st in stages[:2])
            left = run_stages(stages[2:], left, prep_wo() + take(nk))
        else:
            left = run_stages(k_stages(a_s), halo(k_s) + left, merge(mix_a, take(nk)))
        if b == 2:
            wait(w2, x_copy(3))
        left = run_stages(q_stages(a_s), left, merge(mix_b, take(nq)), lead)
        if b == 1:
            wait(w1[1], w1[2])
        if last:
            wait(fence)
        sc_a, sc_b = cut(scores(False), tune["last_scores" if last else "scores"])
        stats, forms = ([], []) if last else (flat(x) for x in norm1((b + 1) * TM, a_s))
        left = run_stages(v_stages(a_s), halo(v_s) + left, merge(sc_a, stats, take(nv)))
        if not last:
            left = run_stages(o_stages(b - 1, o_s), left, merge(
                sc_b, forms, first_stats if b == 2 else [], take(no)), lead)
    mix_a, mix_b = cut(mix(a_s), tune["last_mix"])
    forms_a, forms_b = cut(first_forms, tune["first_forms"])
    left = run_stages(o_stages(NB - 2, o_s), left,
                      merge(sc_b + merge(mix_a, forms_a), take(no)), lead)
    early, late = o_stages(NB - 1, a_s, halves=True, park=False)
    run_stages(early, left, merge(mix_b, forms_b, take(tune["weights"][-2])), lead)
    run(run_stages(late, [], take(tune["weights"][-1]), lead))
    assert not jobs

    def ffn_step(i, carry):
        row0 = pl.multiple_of(i * TM, TM)
        nxt = pl.multiple_of(jnp.minimum(i + 1, NB - 1) * TM, TM)
        prev = pl.multiple_of((i + NB - 1) % NB * TM, TM)
        hold.reset(i)
        left = run_stages(expand(), contract(prev, 1)[0][1], [])
        one, two = contract(row0, 0)
        interleave(one[0], left)
        norm_a, norm_b = cut(flat(flat(x) for x in norm2(nxt)), tune["norm"])
        left = run_stages([two], [], norm_a)
        dots = contract(row0, 1)[0][0]
        n = int(TWO.p * tune["send"]) * 3
        interleave(dots[:n], merge(left, norm_b), lead=tune["out_lead"])

        def send(k):
            pl.when(k == 1)(out_copy(row0, TM, 0, 2 * i).start)
            pl.when(k == 0)(out_copy(prev, TM, 1, jnp.maximum(2 * i - 1, 0)).start)
        each(jnp.where(i > 0, 0, 1), 2, send)
        run([(d, 0) for d in dots[n:]])
        return carry

    lax.fori_loop(0, NB, ffn_step, 0)
    hold.latest = None
    tail = [out_copy(S - TM + 128 * u, 128, 1, 2 * NB - 1 + u) for u in range(4)]
    for tasks, c in zip(split(contract(S - TM, 1)[0][1], 4), tail):
        run(tasks)
        c.start()
    for c in [out_copy(n // 2 * TM, TM, n % 2, n) for n in range(2 * NB - 1)] + tail:
        c.wait()


@jax.jit
def pallas_sequential_preLN__sliding_local_dilated__dense_activation_silu__prompt_kernel(
    A_x: jax.Array,
    A_wqkv: jax.Array,
    A_wo: jax.Array,
    B_x: jax.Array,
    B_w1: jax.Array,
    B_w2: jax.Array,
):
    del B_x
    scratch = [
        pltpu.VMEM((S, D), BF),
        pltpu.VMEM((8, S, 128), F32),
        pltpu.VMEM((36, 128, D), BF),
        pltpu.VMEM((D, F), BF),
        pltpu.VMEM(ONE.forms(D, D), BF),
        pltpu.VMEM(ONE.forms(D, D), BF),
        pltpu.VMEM(ONE.forms(D, D), BF),
        pltpu.VMEM(ONE.forms(D, D), BF),
        pltpu.VMEM((NCH,) + TWO.forms(D, 512), BF),
        pltpu.VMEM((NCH,) + TWO.forms(512, D), BF),
        pltpu.VMEM((8, TM, 128), F32),
        pltpu.VMEM((8, HALO + TM, 128), F32),
        pltpu.VMEM((8, HALO + TM, 128), F32),
        pltpu.VMEM((WIN, TM, 128), F32),
        pltpu.VMEM(ONE.forms(TM, D), BF),
        pltpu.VMEM(TWO.forms(TM, F), BF),
        pltpu.VMEM((16, D), BF),
        pltpu.SemaphoreType.DMA((NB + 1,)),
        pltpu.SemaphoreType.DMA((9,)),
        pltpu.SemaphoreType.DMA((4,)),
        pltpu.SemaphoreType.DMA((2 * NB + 3,)),
        pltpu.VMEM(ONE.forms(TM, D), BF),
        pltpu.VMEM(TWO.forms(TM, D), BF),
    ]
    out = pl.pallas_call(
        kernel,
        in_specs=[pl.BlockSpec(memory_space=pl.ANY)] * 5,
        out_specs=pl.BlockSpec(memory_space=pl.ANY),
        out_shape=jax.ShapeDtypeStruct((S, D), BF),
        scratch_shapes=scratch,
        compiler_params=pltpu.CompilerParams(vmem_limit_bytes=126 << 20),
    )(A_x.reshape(S, D), A_wqkv.reshape(8, 128, 3 * D), A_wo.reshape(8, 128, D),
      B_w1, B_w2.reshape(F // 128, 128, D))
    return out.reshape(1, S, D)
```

```python
import functools

import jax
import jax.numpy as jnp
from jax import lax
import jax.experimental.pallas as pl
import jax.experimental.pallas.tpu as pltpu

BF = jnp.bfloat16
F32 = jnp.float32
U32 = jnp.uint32

S, D, F = 2048, 1024, 3584
WIN, DIL, DH = 8, 2, 32
EPS = 1e-5
SCALE = DH ** -0.5
LOG2E = 1.4426950408889634

TM = 512
NB = S // TM
NCH = F // 512
HALO = 16

TUNE = dict(
    first_scores=0.4, scores=0.9, last_scores=1.0,
    mix=0.55, last_mix=0.8, early_forms=0.4, first_forms=0.5, norm=0.6,
    weights=(1, 0, 0, 1, 2, 3, 0, 0, 2, 3, 0, 0, 1, 1),
    q_lead=0.99, v_lead=1.06, lead=1.05, first_lead=1.2, out_lead=1.2,
    early_products=16, send=0.85, silu_cost=14,
)


def _quad(g):
    n = len(g) // 2
    return ([r[:n] for r in g[:n]], [r[n:] for r in g[:n]],
            [r[:n] for r in g[n:]], [r[n:] for r in g[n:]])


def _add(a, b):
    return [[x + y for x, y in zip(r, s)] for r, s in zip(a, b)]


def _sub(a, b):
    return [[x - y for x, y in zip(r, s)] for r, s in zip(a, b)]


def lhs_forms(g):
    if len(g) == 1:
        yield g[0][0]
        return
    a11, a12, a21, a22 = _quad(g)
    yield from lhs_forms(_add(a11, a22))
    yield from lhs_forms(_add(a21, a22))
    yield from lhs_forms(a11)
    yield from lhs_forms(a22)
    yield from lhs_forms(_add(a11, a12))
    yield from lhs_forms(_sub(a21, a11))
    yield from lhs_forms(_sub(a12, a22))


def rhs_forms(g):
    if len(g) == 1:
        yield g[0][0]
        return
    b11, b12, b21, b22 = _quad(g)
    yield from rhs_forms(_add(b11, b22))
    yield from rhs_forms(b11)
    yield from rhs_forms(_sub(b12, b22))
    yield from rhs_forms(_sub(b21, b11))
    yield from rhs_forms(b22)
    yield from rhs_forms(_add(b11, b12))
    yield from rhs_forms(_add(b21, b22))


def out_forms(get, lo, count):
    if count == 1:
        return [[get(lo)]]
    c = count // 7
    m1 = yield from out_forms(get, lo, c)
    m2 = yield from out_forms(get, lo + c, c)
    c22 = _sub(m1, m2)
    m3 = yield from out_forms(get, lo + 2 * c, c)
    c22 = _add(c22, m3)
    m4 = yield from out_forms(get, lo + 3 * c, c)
    c21 = _add(m2, m4)
    c11 = _add(m1, m4)
    m5 = yield from out_forms(get, lo + 4 * c, c)
    c12 = _add(m3, m5)
    c11 = _sub(c11, m5)
    m6 = yield from out_forms(get, lo + 5 * c, c)
    c22 = _add(c22, m6)
    m7 = yield from out_forms(get, lo + 6 * c, c)
    c11 = _add(c11, m7)
    if count == 7:
        yield
    return [r + s for r, s in zip(c11, c12)] + [r + s for r, s in zip(c21, c22)]


def emit_forms(left, n, get, put):
    forms = lhs_forms if left else rhs_forms
    if n < 4:
        for i, f in enumerate(forms([[get(r, c) for c in range(n)] for r in range(n)])):
            put(i, f.astype(BF))
        return

    def quad(r, c):
        return [[get(2 * r + i, 2 * c + j) for j in range(2)] for i in range(2)]

    def group(g, grid):
        for i, f in enumerate(forms(grid)):
            put(7 * g + i, f.astype(BF))

    x11 = quad(0, 0)
    yield
    group(2 if left else 1, x11)
    yield
    x22 = quad(1, 1)
    yield
    group(3 if left else 4, x22)
    yield
    group(0, _add(x11, x22))
    yield
    x12 = quad(0, 1)
    yield
    group(4 if left else 5, _add(x11, x12))
    yield
    group(6 if left else 2, _sub(x12, x22))
    yield
    x21 = quad(1, 0)
    yield
    group(1 if left else 6, _add(x21, x22))
    yield
    group(5 if left else 3, _sub(x21, x11))


def form_costs(n, fetch):
    q = 4 * fetch
    return [q, 17, q, 17, 25, q, 25, 25, q, 25, 25] if n == 4 else [q + 17]


class Split:
    def __init__(self, level):
        self.n = 2 ** level
        self.p = 7 ** level
        self.sub = 4 // self.n
        self.slabs = TM // 16 // self.n

    def slab(self, g, t):
        per = 8 // self.n
        return 8 * (t // per) + per * g + t % per

    def tile(self, c, a):
        return 4 * (a // self.sub) + self.sub * c + a % self.sub

    def forms(self, rows, cols):
        return (self.p, cols // self.n // 128, rows // self.n, 128)


ONE, TWO = Split(1), Split(2)


def mm(a, b):
    return jnp.dot(pltpu.bitcast(a, BF), pltpu.bitcast(b, BF),
                   preferred_element_type=F32)


def tile(x, j):
    return x[:, 128 * j:128 * (j + 1)]


def cat(xs, axis):
    return xs[0] if len(xs) == 1 else jnp.concatenate(xs, axis=axis)


def skew(xs, step, axis):
    return [x if t == 0 else pltpu.roll(x, t * step, axis) for t, x in enumerate(xs)]


def unskew(xs, step, axis):
    n = len(xs)
    size = xs[0].shape[axis]
    field = lax.broadcasted_iota(jnp.int32, xs[0].shape, axis) // step
    zs = [xs[-i % n] for i in range(n)]
    b = 1
    while b < n:
        bit = (field & b) != 0
        zs = [jnp.where(bit, zs[(i - b) % n], zs[i]) for i in range(n)]
        b *= 2
    return [z if j == 0 else pltpu.roll(z, size - j * step, axis)
            for j, z in enumerate(zs)]


def silu(x):
    h = 0.5 * x
    return h + h * jnp.tanh(h)


def staged(gen, costs):
    def step(last):
        next(gen, None)
        if last:
            assert next(gen, "done") == "done"
    return [(functools.partial(step, k == len(costs) - 1), c)
            for k, c in enumerate(costs)]


def run(tasks):
    for fn, _ in tasks:
        fn()


def merge(*lists):
    keyed = []
    for n, lst in enumerate(lists):
        total = sum(c for _, c in lst)
        acc = 0
        for item in lst:
            keyed.append(((acc + item[1] / 2) / total, n, item))
            acc += item[1]
    keyed.sort(key=lambda e: e[:2])
    return [e[2] for e in keyed]


def diagonal(pieces):
    depth = len(pieces[0])
    return [task for n in range(len(pieces) + depth - 1)
            for task in merge(*[pieces[n - k][k] for k in range(depth)
                                if 0 <= n - k < len(pieces)])]


def overlap(first, second):
    return diagonal(list(zip(first, second)))


def split(tasks, parts):
    total = sum(c for _, c in tasks)
    out = [[] for _ in range(parts)]
    acc = 0
    for item in tasks:
        out[min(int((acc + item[1] / 2) * parts / max(total, 1)), parts - 1)].append(item)
        acc += item[1]
    return out


def cut(tasks, share):
    n = int(len(tasks) * share)
    return tasks[:n], tasks[n:]


def each(lo, hi, fn):
    def body(i, carry):
        fn(i)
        return i
    return lax.fori_loop(lo, hi, body, jnp.int32(0))


class Pace:
    def __init__(self):
        self.never = self.latest = None
        self.phase = 0

    def reset(self, index):
        self.never, self.latest = index < 0, None

    def mark(self, product):
        self.latest = product

    def __call__(self, x):
        if self.latest is None:
            return x
        n = x.shape[0] * x.dtype.itemsize // 4
        row = min(8 * int(self.phase * self.latest.shape[0] / 8), self.latest.shape[0] - n)
        other = self.latest[row:row + n]
        if x.dtype == BF:
            other = pltpu.bitcast(other, BF)
        return jnp.where(self.never, other, x)

    def interleave(self, main, side, lead=1.0):
        total = sum(c for _, c in side)
        step = total * lead / len(main)
        done = i = 0
        for k, fn in enumerate(main):
            fn()
            start = total * lead * k / len(main)
            while i < len(side) and done + side[i][1] / 2 <= start + step:
                self.phase = min(max((done - start) / max(step, 1), 0), 1)
                side[i][0]()
                done += side[i][1]
                i += 1
        run(side[i:])


def kernel(x_hbm, wqkv_hbm, wo_hbm, w1_hbm, w2_hbm, out_hbm,
           x_s, h_s, raw_s, raw1_s, wk_s, wq_s, wv_s, wo_s, w1_s, w2_s,
           q_s, k_s, v_s, p_s, o_s, t_s, pad_s,
           x_sem, raw_sem, w_sem, out_sem, a_s, b_s):
    tune = TUNE
    hold = Pace()
    interleave = hold.interleave

    def x_copy(b):
        rows = pl.ds(b * TM, TM)
        return pltpu.make_async_copy(x_hbm.at[rows], x_s.at[rows], x_sem.at[b])

    def raw_copy(m, tiles, sem, rows=slice(None)):
        return pltpu.make_async_copy(
            wqkv_hbm.at[pl.ds(*tiles), rows, pl.ds(D * (1, 0, 2)[m], D)],
            raw_s.at[pl.ds(8 * m + tiles[0], tiles[1]), rows], raw_sem.at[sem])

    def w1_copy(lo, hi):
        cols = (slice(None), pl.ds(512 * lo, 512 * (hi - lo)))
        return pltpu.make_async_copy(w1_hbm.at[cols], raw1_s.at[cols], w_sem.at[lo])

    def out_copy(row, rows, half, sem):
        idx = (pl.ds(row, rows), pl.ds(512 * half, 512))
        return pltpu.make_async_copy(x_s.at[idx], out_hbm.at[idx], out_sem.at[sem])

    def wait(*copies, start=()):
        def go(n):
            for k, c in enumerate(start):
                pl.when(n == k)(c.start)
            for c in copies:
                pl.when(n == len(start))(c.wait)
        hold.reset(each(0, max(len(start) + 1, 2), go))

    def rhs_square(sp, load, put):
        return [x for ka in range(sp.sub) for na in range(sp.sub) for x in staged(
            emit_forms(False, sp.n,
                       lambda r, c, ka=ka, na=na: hold(load(
                           sp.tile(r, ka), sp.tile(c, na))).astype(F32),
                       lambda i, val, ka=ka, na=na: put(i, ka, na, val)),
            form_costs(sp.n, 4))]

    def proj_square(w_s, kc, s, a, load):
        def put(i, ka, na, val):
            w_s[i, 2 * a + na, pl.ds(128 * (2 * kc + ka) + 16 * s, 16), :] = val
        return rhs_square(ONE, load, put)

    def prep_qkv(m, w_s, halves=(0, 1), slabs=range(8)):
        def permute(kc, s, r):
            w = cat([pltpu.bitcast(raw_s[8 * m + 4 * kc + r + e, pl.ds(16 * s, 16), :], U32)
                     for e in range(2)], 0)
            xs = skew([tile(w, t) for t in range(8)], 4, 1)
            yield
            xs = unskew(xs, 4, 1)
            yield
            for c, x in enumerate(xs):
                p_s[c, pl.ds(256 * kc + 32 * s + 8 * r, 16), :] = pltpu.bitcast(x, F32)

        tasks = []
        for kc in halves:
            pieces = []
            for s in slabs:
                for a in range(2):
                    x, y, z = staged(permute(kc, s, 2 * a), [32, 52, 16])
                    pieces.append([[x], [], [], [y], [], [], [z], [], proj_square(
                        w_s, kc, s, a, lambda r, c, s=s, a=a, kc=kc: pltpu.bitcast(
                            p_s[4 * a + c, pl.ds(256 * kc + 32 * s + 8 * r, 8), :], BF))])
            tasks += diagonal(pieces)
        return tasks

    def prep_wo():
        tasks = []
        for kc in range(2):
            for s in range(8):
                for a in range(2):
                    rows = []

                    def fetch(kc=kc, s=s, a=a, rows=rows):
                        hh, t2 = divmod(s, 2)
                        rows.extend(unskew(skew([pltpu.bitcast(raw_s[
                            28 + 4 * t2 + t, pl.ds(32 * hh + 16 * kc, 16),
                            pl.ds(512 * a, 512)], U32) for t in range(4)], 2, 0), 2, 0))
                    tasks.append((fetch, 70))
                    tasks += proj_square(
                        wo_s, kc, s, a,
                        lambda r, c, rows=rows: pltpu.bitcast(tile(rows[r], c), BF))
        return tasks

    def prep_w1(j):
        def square(kc, s):
            def put(i, ka, na, val):
                w1_s[j, i, 0, pl.ds(128 * kc + 16 * s, 16), :] = val
            return rhs_square(TWO, lambda r, c: raw1_s[
                pl.ds(512 * kc + 128 * r + 16 * s, 16), pl.ds(512 * j + 128 * c, 128)], put)
        return [x for kc in range(2) for s in range(8) for x in square(kc, s)]

    def prep_w2(j):
        def square(a, s):
            def put(i, ka, na, val):
                w2_s[j, i, a, pl.ds(16 * s, 16), :] = val
            return rhs_square(TWO, lambda r, c: raw_s[
                4 * j + r, pl.ds(16 * s, 16), pl.ds(512 * a + 128 * c, 128)], put)
        return [x for a in range(2) for s in range(8) for x in square(a, s)]

    def moments(load, out):
        x = [load(j) for j in range(8)]
        mean = jnp.sum(functools.reduce(jnp.add, x), axis=-1, keepdims=True) * (1.0 / D)
        yield
        x = [t - mean for t in x]
        sq = functools.reduce(jnp.add, [t * t for t in x])
        var = jnp.sum(sq, axis=-1, keepdims=True) * (1.0 / D)
        yield
        inv = lax.rsqrt(var + EPS)
        out.append(lambda j: hold(x[j]) * inv)

    def norm(sp, load, dst, first_cost):
        stats, forms = [], []
        for t in range(sp.slabs):
            rows = [[] for _ in range(sp.n)]
            stats.append(merge(*[staged(moments(
                functools.partial(load, 16 * sp.slab(g, t)), rows[g]), [first_cost, 46, 10])
                for g in range(sp.n)]))

            def put(i, val, a, t=t):
                dst[i, a, pl.ds(16 * t, 16), :] = val
            forms.append([x for a in range(8 // sp.n) for x in staged(
                emit_forms(True, sp.n,
                           lambda r, c, a=a, rows=rows: rows[r][0](sp.tile(c, a)),
                           functools.partial(put, a=a)),
                form_costs(sp.n, 4))])
        return stats, forms

    def norm1(row0, dst):
        return norm(ONE, lambda r, j: hold(
            x_s[pl.ds(row0 + r, 16), pl.ds(128 * j, 128)]).astype(F32), dst, 38)

    def norm2(row0):
        return norm(TWO, lambda r, j: hold(h_s[j, pl.ds(row0 + r, 16), :]), b_s, 30)

    def project(lhs_s, w_s, sink, halves=False, park=True):
        stages, early = [], []
        for a0 in (0, 2):
            for r in range(2):
                m = {}

                def dot(i, k, a0=a0, r=r, m=m):
                    d = mm(cat([lhs_s.bitcast(U32)[i, 2 * k + c, pl.ds(64 * r, 64), :]
                                for c in range(2)], 1),
                           cat([w_s.bitcast(U32)[i, a0 + a, pl.ds(128 * k, 128), :]
                                for a in range(2)], 1))
                    hold.mark(tile(d, 0))
                    for a in range(2):
                        n = ((a0 + a) * 7 + i) * 256 + 128 * r
                        spot = (n // S, pl.ds(n % S, 128))
                        if halves and park and k == 0:
                            h_s[spot] = tile(d, a)
                        elif halves and park:
                            m[a, i] = h_s[spot] + tile(d, a)
                        else:
                            m[a, i] = tile(d, a) if k == 0 else m[a, i] + tile(d, a)

                def post(t, a, a0=a0, r=r, m=m):
                    c = yield from out_forms(lambda i: m[a, i][16 * t:16 * t + 16], 0, 7)
                    for g in range(2):
                        for cc in range(2):
                            sink(ONE.tile(cc, a0 + a), ONE.slab(g, 8 * r + t), c[g][cc])

                posts = [x for a in range(2) for t in range(8)
                         for x in staged(post(t, a), [18, 10])]
                if halves:
                    early.append(([functools.partial(dot, i, 0) for i in range(7)], []))
                stages.append(([functools.partial(dot, i, k) for i in range(7)
                                for k in ((1,) if halves else (0, 1))], posts))
        return (early, stages) if halves else stages

    def run_stages(stages, carried, side, lead=1.0):
        idle = sum(c for _, c in side) * (lead - 1)
        side = side + [(lambda: None, idle / 8)] * 8
        for (dots, posts), part in zip(stages, split(side, len(stages))):
            interleave(dots, carried + part)
            carried = posts
        return carried

    def to_ref(ref, off):
        def sink(j, sl, val):
            ref[j, pl.ds(off + 16 * sl, 16), :] = val
        return sink

    def residual(row0):
        def sink(j, sl, val):
            rows = pl.ds(row0 + 16 * sl, 16)
            h_s[j, rows, :] = hold(x_s[rows, pl.ds(128 * j, 128)]).astype(F32) + val
        return sink

    def scores(first_block):
        lane = lax.broadcasted_iota(jnp.int32, (8, 128), 1)
        odd, high = (lane & 1) != 0, (lane & 2) != 0
        up = lambda x, b: pltpu.roll(x, b, 1)
        down = lambda x, b: pltpu.roll(x, 128 - b, 1)

        def go(r):
            acc = [None] * WIN
            for j in range(8):
                q = hold(q_s[j, pl.ds(r, 8), :])
                for w in range(WIN):
                    kw = k_s[j, pl.ds(HALO + r - DIL * w, 8), :]
                    acc[w] = q * kw if j == 0 else acc[w] + q * kw
                if j % 2:
                    yield
            xs = [(acc[w], up(acc[w], 1), acc[w + 1], down(acc[w + 1], 1))
                  for w in range(0, WIN, 2)]
            yield
            xs = [jnp.where(odd, a + ua, b + db) for a, ua, b, db in xs]
            xs = [hold(x) for x in xs]
            xs = [(x, up(x, 2), down(x, 2)) for x in xs]
            yield
            logit = [x + jnp.where(high, u, d) for x, u, d in xs]
            if first_block and r < DIL * (WIN - 1):
                row = lax.broadcasted_iota(jnp.int32, (8, 128), 0) + r
                for n, s in enumerate(logit):
                    w = jnp.where(odd, 2 * n, 2 * n + 1)
                    logit[n] = jnp.where(row >= DIL * w, s * SCALE, -1e9)
                factor = LOG2E
            else:
                factor = SCALE * LOG2E
            top = functools.reduce(jnp.maximum, logit)
            u, d = up(top, 1), down(top, 1)
            yield
            top = jnp.maximum(top, jnp.where(odd, u, d))
            e = [jnp.exp2((s - top) * factor) for s in logit]
            total = functools.reduce(jnp.add, e)
            u, d = up(total, 1), down(total, 1)
            yield
            inv = 1.0 / (total + jnp.where(odd, u, d))
            e = [x * inv for x in e]
            xs = [(x, up(x, 1), down(x, 1)) for x in e]
            yield
            e = [y for x, u, d in xs for y in (jnp.where(odd, x, d), jnp.where(odd, u, x))]
            for w in range(WIN):
                p_s[w, pl.ds(r, 8), :] = e[w]

        pieces = [staged(go(r), [32] * 4 + [8, 20, 12, 16, 16, 16]) for r in range(0, TM, 8)]
        return [task for n in range(len(pieces) + 6) for task in merge(
            pieces[n][:4] if n < len(pieces) else [],
            [pieces[n - k][3 + k] for k in range(1, 7) if 0 <= n - k < len(pieces)])]

    def mix(dst):
        def go(t, a):
            grid = [[], []]
            for g in range(2):
                r = 16 * ONE.slab(g, t)
                p = [hold(p_s[w, pl.ds(r, 16), :]) for w in range(WIN)]
                for c in range(2):
                    terms = []
                    for w in range(WIN // 2):
                        v = v_s[ONE.tile(c, a), pl.ds(HALO + r - DIL * w - 8, 24), :]
                        terms.append(p[w] * v[8:] + p[w + 4] * v[:16])
                    grid[g].append((terms[0] + terms[1]) + (terms[2] + terms[3]))
                    yield

            def put(i, val):
                dst[i, a, pl.ds(16 * t, 16), :] = val
            yield from emit_forms(True, 2, lambda g, c: grid[g][c], put)

        return [x for lo in (0, 2) for t in range(ONE.slabs) for a in (lo, lo + 1)
                for x in staged(go(t, a), [46, 30, 46, 30, 17])]

    def halo(ref):
        def keep():
            ref[:, pl.ds(0, HALO), :] = ref[:, pl.ds(TM, HALO), :]
        return [(keep, 0)]

    def first_halo():
        for j in range(8):
            v_s[j, pl.ds(0, HALO), :] = jnp.broadcast_to(
                v_s[j, pl.ds(HALO, 1), :], (HALO, 128))

    def expand():
        stages = []
        for j in range(NCH):
            m = [None] * TWO.p

            def dot(p, j=j, m=m):
                m[p] = mm(cat([b_s.bitcast(U32)[p, c] for c in range(2)], 1),
                          w1_s.bitcast(U32)[j, p, 0])
                hold.mark(m[p])

            def post(t, j=j, m=m):
                c = yield from out_forms(lambda p: m[p][16 * t:16 * t + 16], 0, TWO.p)

                def put(p, val):
                    t_s[p, j, pl.ds(16 * t, 16), :] = val
                yield from emit_forms(True, 4, lambda g, cc: silu(hold(c[g][cc])), put)

            stages.append(([functools.partial(dot, p) for p in range(TWO.p)],
                           [x for t in range(TWO.slabs) for x in staged(
                               post(t), [0] * 7 + form_costs(4, tune["silu_cost"]))]))
        return stages

    def parked(p, rows=slice(None)):
        ref, start = (q_s, p_s)[p // 32], 128 * (p % 4)
        lo, hi, _ = rows.indices(128)
        return ref, (p % 32 // 4, pl.ds(start + lo, hi - lo))

    def contract(row0, a):
        m = [None] * TWO.p

        def dot(p, j0, j1):
            d = mm(cat([t_s.bitcast(U32)[p, j] for j in range(j0, j1)], 1),
                   cat([w2_s.bitcast(U32)[j, p, a] for j in range(j0, j1)], 0))
            m[p] = d if m[p] is None else m[p] + d
            hold.mark(d)
            if a and j1 == NCH:
                ref, idx = parked(p)
                ref[idx] = m[p]

        def product(p, t):
            if not a:
                return m[p][16 * t:16 * t + 16]
            ref, idx = parked(p, slice(16 * t, 16 * t + 16))
            return hold(ref[idx])

        def post(t):
            c = yield from out_forms(lambda p: product(p, t), 0, TWO.p)
            for g in range(4):
                rows = pl.ds(row0 + 16 * TWO.slab(g, t), 16)
                x_s[rows, pl.ds(512 * a, 512)] = cat(
                    [h_s[4 * a + cc, rows, :] + (c[g][cc] if a else hold(c[g][cc]))
                     for cc in range(4)], 1).astype(BF)
                if g == 1:
                    yield

        def dots(products, *edges):
            return [functools.partial(dot, p, j0, j1) for p in products
                    for j0, j1 in zip(edges, edges[1:])]

        posts = [x for t in range(TWO.slabs)
                 for x in staged(post(t), [30 if a else 0] * 7 + [36] * 2)]
        if a:
            return [(dots(range(TWO.p), 0, 2, 4, NCH), posts)]
        n = tune["early_products"]
        return [(dots(range(n), 0, 2, 4, NCH - 1), []),
                (dots(range(n), NCH - 1, NCH) + dots(range(n, TWO.p), 0, 2, 4, NCH), posts)]

    k_stages = lambda lhs, **kw: project(lhs, wk_s, to_ref(k_s, HALO), **kw)
    q_stages = lambda lhs, **kw: project(lhs, wq_s, to_ref(q_s, 0), **kw)
    v_stages = lambda lhs: project(lhs, wv_s, to_ref(v_s, HALO))
    o_stages = lambda b, lhs, **kw: project(lhs, wo_s, residual(b * TM), **kw)
    flat = lambda parts: [x for part in parts for x in part]
    lead, q_lead, v_lead = tune["lead"], tune["q_lead"], tune["v_lead"]

    jobs = [f(j) for f in (prep_w1, prep_w2) for j in range(NCH)]
    take = lambda n: flat([jobs.pop(0) for _ in range(n)])
    first_stats, first_forms = (flat(x) for x in norm2(0))

    head = [raw_copy(0, (0, 4), h, pl.ds(64 * h, 64)) for h in range(2)]
    k1 = [raw_copy(0, (4, 4), 2 + 7 * h, pl.ds(64 * h, 64)) for h in range(2)]
    q0, q1, v0, v1 = (raw_copy(m, (4 * kc, 4), 2 * m + kc + 1)
                      for m in (1, 2) for kc in range(2))
    x0 = [pltpu.make_async_copy(x_hbm.at[pl.ds(256 * r, 256)], x_s.at[pl.ds(256 * r, 256)],
                                x_sem.at[NB * r]) for r in range(2)]
    wo = pltpu.make_async_copy(wo_hbm, raw_s.at[pl.ds(28, 8)], raw_sem.at[7])
    w1 = [w1_copy(0, 1), w1_copy(1, 2), w1_copy(2, NCH)]
    w2 = pltpu.make_async_copy(w2_hbm, raw_s.at[pl.ds(0, 28)], w_sem.at[3])
    fence = pltpu.make_async_copy(wo_hbm.at[0, pl.ds(0, 16)], pad_s, raw_sem.at[8])

    wait(x0[0], start=[x0[0], *head, x0[1], *k1, q0, q1, v0, x_copy(1), v1,
                       wo, x_copy(2), w1[0]])
    k_s[:, pl.ds(0, HALO), :] = jnp.zeros((8, HALO, 128), F32)
    stats, forms = norm1(0, o_s)
    run(overlap(stats[:8], forms[:8]))
    for h in range(2):
        wait(head[h])
        run(prep_qkv(0, wk_s, (0,), range(4 * h, 4 * h + 4)))
    early, late = k_stages(o_s, halves=True)
    dots = flat(early[n][0] for n in (0, 2, 1, 3))
    x0[1].wait()
    interleave(dots[:12], overlap(stats[8:], forms[8:]), lead=1.0)
    for h, part in enumerate((dots[12:20], dots[20:])):
        k1[h].wait()
        interleave(part, prep_qkv(0, wk_s, (1,), range(4 * h, 4 * h + 4)), lead=1.0)
    run([(d, 0) for st in late[:2] for d in st[0]])
    q0.wait()
    left = run_stages(late[2:], flat(st[1] for st in late[:2]), prep_qkv(1, wq_s, (0,)), q_lead)
    wait(q1)
    early, late = q_stages(o_s, halves=True)
    run_stages(early, left, prep_qkv(1, wq_s, (1,)), q_lead)
    wait(v0, x_copy(1))
    stats, forms = (flat(x) for x in norm1(TM, a_s))
    left = run_stages(late, [], merge(prep_qkv(2, wv_s, (0,)), stats), v_lead)
    wait(v1, start=[w1[1], w1[2]])
    early, late = project(o_s, wv_s, to_ref(v_s, HALO), halves=True, park=False)
    sc_a, sc_b = cut(scores(True), tune["first_scores"])
    forms_a, forms_b = cut(forms, tune["early_forms"])
    run_stages(early, left, merge(prep_qkv(2, wv_s, (1,)), forms_a), v_lead)
    left = run_stages(late, [], merge(sc_a, forms_b), tune["first_lead"])

    for b in range(1, NB):
        last = b == NB - 1
        nk, nq, nv, no = tune["weights"][4 * b - 4:4 * b]
        mix_a, mix_b = cut(mix(o_s), 0.0 if b == 1 else tune["mix"])
        if b == 1:
            wait(wo, x_copy(2), w1[0], start=[w2, x_copy(3), fence])
            stages = k_stages(a_s)
            interleave(flat(st[0] for st in stages[:2]), merge(left, sc_b), lead=1.1)
            left = [(first_halo, 0)] + halo(k_s) + flat(st[1] for st in stages[:2])
            left = run_stages(stages[2:], left, prep_wo() + take(nk))
        else:
            left = run_stages(k_stages(a_s), halo(k_s) + left, merge(mix_a, take(nk)))
        if b == 2:
            wait(w2, x_copy(3))
        left = run_stages(q_stages(a_s), left, merge(mix_b, take(nq)), lead)
        if b == 1:
            wait(w1[1], w1[2])
        if last:
            wait(fence)
        sc_a, sc_b = cut(scores(False), tune["last_scores" if last else "scores"])
        stats, forms = ([], []) if last else (flat(x) for x in norm1((b + 1) * TM, a_s))
        left = run_stages(v_stages(a_s), halo(v_s) + left, merge(sc_a, stats, take(nv)))
        if not last:
            left = run_stages(o_stages(b - 1, o_s), left, merge(
                sc_b, forms, first_stats if b == 2 else [], take(no)), lead)
    mix_a, mix_b = cut(mix(a_s), tune["last_mix"])
    forms_a, forms_b = cut(first_forms, tune["first_forms"])
    left = run_stages(o_stages(NB - 2, o_s), left,
                      merge(sc_b + merge(mix_a, forms_a), take(no)), lead)
    early, late = o_stages(NB - 1, a_s, halves=True, park=False)
    run_stages(early, left, merge(mix_b, forms_b, take(tune["weights"][-2])), lead)
    run(run_stages(late, [], take(tune["weights"][-1]), lead))
    assert not jobs

    def ffn_step(i, carry):
        row0 = pl.multiple_of(i * TM, TM)
        nxt = pl.multiple_of(jnp.minimum(i + 1, NB - 1) * TM, TM)
        prev = pl.multiple_of((i + NB - 1) % NB * TM, TM)
        hold.reset(i)
        left = run_stages(expand(), contract(prev, 1)[0][1], [])
        one, two = contract(row0, 0)
        interleave(one[0], left)
        norm_a, norm_b = cut(flat(flat(x) for x in norm2(nxt)), tune["norm"])
        left = run_stages([two], [], norm_a)
        dots = contract(row0, 1)[0][0]
        n = int(TWO.p * tune["send"]) * 3
        interleave(dots[:n], merge(left, norm_b), lead=tune["out_lead"])

        def send(k):
            pl.when(k == 1)(out_copy(row0, TM, 0, 2 * i).start)
            pl.when(k == 0)(out_copy(prev, TM, 1, jnp.maximum(2 * i - 1, 0)).start)
        each(jnp.where(i > 0, 0, 1), 2, send)
        run([(d, 0) for d in dots[n:]])
        return carry

    lax.fori_loop(0, NB, ffn_step, 0)
    hold.latest = None
    tail = [out_copy(S - TM + 128 * u, 128, 1, 2 * NB - 1 + u) for u in range(4)]
    for tasks, c in zip(split(contract(S - TM, 1)[0][1], 4), tail):
        run(tasks)
        c.start()
    for c in [out_copy(n // 2 * TM, TM, n % 2, n) for n in range(2 * NB - 1)] + tail:
        c.wait()


@jax.jit
def pallas_sequential_preLN__sliding_local_dilated__dense_activation_silu__prompt_kernel(
    A_x: jax.Array,
    A_wqkv: jax.Array,
    A_wo: jax.Array,
    B_x: jax.Array,
    B_w1: jax.Array,
    B_w2: jax.Array,
):
    del B_x
    scratch = [
        pltpu.VMEM((S, D), BF),
        pltpu.VMEM((8, S, 128), F32),
        pltpu.VMEM((36, 128, D), BF),
        pltpu.VMEM((D, F), BF),
        pltpu.VMEM(ONE.forms(D, D), BF),
        pltpu.VMEM(ONE.forms(D, D), BF),
        pltpu.VMEM(ONE.forms(D, D), BF),
        pltpu.VMEM(ONE.forms(D, D), BF),
        pltpu.VMEM((NCH,) + TWO.forms(D, 512), BF),
        pltpu.VMEM((NCH,) + TWO.forms(512, D), BF),
        pltpu.VMEM((8, TM, 128), F32),
        pltpu.VMEM((8, HALO + TM, 128), F32),
        pltpu.VMEM((8, HALO + TM, 128), F32),
        pltpu.VMEM((WIN, TM, 128), F32),
        pltpu.VMEM(ONE.forms(TM, D), BF),
        pltpu.VMEM(TWO.forms(TM, F), BF),
        pltpu.VMEM((16, D), BF),
        pltpu.SemaphoreType.DMA((NB + 1,)),
        pltpu.SemaphoreType.DMA((10,)),
        pltpu.SemaphoreType.DMA((4,)),
        pltpu.SemaphoreType.DMA((2 * NB + 3,)),
        pltpu.VMEM(ONE.forms(TM, D), BF),
        pltpu.VMEM(TWO.forms(TM, D), BF),
    ]
    out = pl.pallas_call(
        kernel,
        in_specs=[pl.BlockSpec(memory_space=pl.ANY)] * 5,
        out_specs=pl.BlockSpec(memory_space=pl.ANY),
        out_shape=jax.ShapeDtypeStruct((S, D), BF),
        scratch_shapes=scratch,
        compiler_params=pltpu.CompilerParams(vmem_limit_bytes=126 << 20),
    )(A_x.reshape(S, D), A_wqkv.reshape(8, 128, 3 * D), A_wo.reshape(8, 128, D),
      B_w1, B_w2.reshape(F // 128, 128, D))
    return out.reshape(1, S, D)
```

```python
import functools

import jax
import jax.numpy as jnp
from jax import lax
import jax.experimental.pallas as pl
import jax.experimental.pallas.tpu as pltpu

BF = jnp.bfloat16
F32 = jnp.float32
U32 = jnp.uint32

S, D, F = 2048, 1024, 3584
WIN, DIL, DH = 8, 2, 32
EPS = 1e-5
SCALE = DH ** -0.5
LOG2E = 1.4426950408889634

TM = 512
NB = S // TM
NCH = F // 512
HALO = 16

TUNE = dict(
    first_scores=0.4, scores=0.9, last_scores=1.0,
    mix=0.55, last_mix=0.8, early_forms=0.4, first_forms=0.5, norm=0.6,
    weights=(1, 0, 0, 1, 2, 3, 0, 0, 2, 3, 0, 0, 1, 1),
    q_lead=0.99, v_lead=1.06, lead=1.02, first_lead=1.2, out_lead=1.2,
    head_cuts=(5, 13, 20), early_products=16, send=0.85, silu_cost=14,
)


def _quad(g):
    n = len(g) // 2
    return ([r[:n] for r in g[:n]], [r[n:] for r in g[:n]],
            [r[:n] for r in g[n:]], [r[n:] for r in g[n:]])


def _add(a, b):
    return [[x + y for x, y in zip(r, s)] for r, s in zip(a, b)]


def _sub(a, b):
    return [[x - y for x, y in zip(r, s)] for r, s in zip(a, b)]


def lhs_forms(g):
    if len(g) == 1:
        yield g[0][0]
        return
    a11, a12, a21, a22 = _quad(g)
    yield from lhs_forms(_add(a11, a22))
    yield from lhs_forms(_add(a21, a22))
    yield from lhs_forms(a11)
    yield from lhs_forms(a22)
    yield from lhs_forms(_add(a11, a12))
    yield from lhs_forms(_sub(a21, a11))
    yield from lhs_forms(_sub(a12, a22))


def rhs_forms(g):
    if len(g) == 1:
        yield g[0][0]
        return
    b11, b12, b21, b22 = _quad(g)
    yield from rhs_forms(_add(b11, b22))
    yield from rhs_forms(b11)
    yield from rhs_forms(_sub(b12, b22))
    yield from rhs_forms(_sub(b21, b11))
    yield from rhs_forms(b22)
    yield from rhs_forms(_add(b11, b12))
    yield from rhs_forms(_add(b21, b22))


def out_forms(get, lo, count):
    if count == 1:
        return [[get(lo)]]
    c = count // 7
    m1 = yield from out_forms(get, lo, c)
    m2 = yield from out_forms(get, lo + c, c)
    c22 = _sub(m1, m2)
    m3 = yield from out_forms(get, lo + 2 * c, c)
    c22 = _add(c22, m3)
    m4 = yield from out_forms(get, lo + 3 * c, c)
    c21 = _add(m2, m4)
    c11 = _add(m1, m4)
    m5 = yield from out_forms(get, lo + 4 * c, c)
    c12 = _add(m3, m5)
    c11 = _sub(c11, m5)
    m6 = yield from out_forms(get, lo + 5 * c, c)
    c22 = _add(c22, m6)
    m7 = yield from out_forms(get, lo + 6 * c, c)
    c11 = _add(c11, m7)
    if count == 7:
        yield
    return [r + s for r, s in zip(c11, c12)] + [r + s for r, s in zip(c21, c22)]


def emit_forms(left, n, get, put):
    forms = lhs_forms if left else rhs_forms
    if n < 4:
        for i, f in enumerate(forms([[get(r, c) for c in range(n)] for r in range(n)])):
            put(i, f.astype(BF))
        return

    def quad(r, c):
        return [[get(2 * r + i, 2 * c + j) for j in range(2)] for i in range(2)]

    def group(g, grid):
        for i, f in enumerate(forms(grid)):
            put(7 * g + i, f.astype(BF))

    x11 = quad(0, 0)
    yield
    group(2 if left else 1, x11)
    yield
    x22 = quad(1, 1)
    yield
    group(3 if left else 4, x22)
    yield
    group(0, _add(x11, x22))
    yield
    x12 = quad(0, 1)
    yield
    group(4 if left else 5, _add(x11, x12))
    yield
    group(6 if left else 2, _sub(x12, x22))
    yield
    x21 = quad(1, 0)
    yield
    group(1 if left else 6, _add(x21, x22))
    yield
    group(5 if left else 3, _sub(x21, x11))


def form_costs(n, fetch):
    q = 4 * fetch
    return [q, 17, q, 17, 25, q, 25, 25, q, 25, 25] if n == 4 else [q + 17]


class Split:
    def __init__(self, level):
        self.n = 2 ** level
        self.p = 7 ** level
        self.sub = 4 // self.n
        self.slabs = TM // 16 // self.n

    def slab(self, g, t):
        per = 8 // self.n
        return 8 * (t // per) + per * g + t % per

    def tile(self, c, a):
        return 4 * (a // self.sub) + self.sub * c + a % self.sub

    def forms(self, rows, cols):
        return (self.p, cols // self.n // 128, rows // self.n, 128)


ONE, TWO = Split(1), Split(2)


def mm(a, b):
    return jnp.dot(pltpu.bitcast(a, BF), pltpu.bitcast(b, BF),
                   preferred_element_type=F32)


def tile(x, j):
    return x[:, 128 * j:128 * (j + 1)]


def cat(xs, axis):
    return xs[0] if len(xs) == 1 else jnp.concatenate(xs, axis=axis)


def skew(xs, step, axis):
    return [x if t == 0 else pltpu.roll(x, t * step, axis) for t, x in enumerate(xs)]


def unskew(xs, step, axis):
    n = len(xs)
    size = xs[0].shape[axis]
    field = lax.broadcasted_iota(jnp.int32, xs[0].shape, axis) // step
    zs = [xs[-i % n] for i in range(n)]
    b = 1
    while b < n:
        bit = (field & b) != 0
        zs = [jnp.where(bit, zs[(i - b) % n], zs[i]) for i in range(n)]
        b *= 2
    return [z if j == 0 else pltpu.roll(z, size - j * step, axis)
            for j, z in enumerate(zs)]


def silu(x):
    h = 0.5 * x
    return h + h * jnp.tanh(h)


def staged(gen, costs):
    def step(last):
        next(gen, None)
        if last:
            assert next(gen, "done") == "done"
    return [(functools.partial(step, k == len(costs) - 1), c)
            for k, c in enumerate(costs)]


def run(tasks):
    for fn, _ in tasks:
        fn()


def merge(*lists):
    keyed = []
    for n, lst in enumerate(lists):
        total = sum(c for _, c in lst)
        acc = 0
        for item in lst:
            keyed.append(((acc + item[1] / 2) / total, n, item))
            acc += item[1]
    keyed.sort(key=lambda e: e[:2])
    return [e[2] for e in keyed]


def diagonal(pieces):
    depth = len(pieces[0])
    return [task for n in range(len(pieces) + depth - 1)
            for task in merge(*[pieces[n - k][k] for k in range(depth)
                                if 0 <= n - k < len(pieces)])]


def overlap(first, second):
    return diagonal(list(zip(first, second)))


def split(tasks, parts):
    total = sum(c for _, c in tasks)
    out = [[] for _ in range(parts)]
    acc = 0
    for item in tasks:
        out[min(int((acc + item[1] / 2) * parts / max(total, 1)), parts - 1)].append(item)
        acc += item[1]
    return out


def cut(tasks, share):
    n = int(len(tasks) * share)
    return tasks[:n], tasks[n:]


def each(lo, hi, fn):
    def body(i, carry):
        fn(i)
        return i
    return lax.fori_loop(lo, hi, body, jnp.int32(0))


class Pace:
    def __init__(self):
        self.never = self.latest = None
        self.phase = 0

    def reset(self, index):
        self.never, self.latest = index < 0, None

    def mark(self, product):
        self.latest = product

    def __call__(self, x):
        if self.latest is None:
            return x
        n = x.shape[0] * x.dtype.itemsize // 4
        row = min(8 * int(self.phase * self.latest.shape[0] / 8), self.latest.shape[0] - n)
        other = self.latest[row:row + n]
        if x.dtype == BF:
            other = pltpu.bitcast(other, BF)
        return jnp.where(self.never, other, x)

    def interleave(self, main, side, lead=1.0):
        total = sum(c for _, c in side)
        step = total * lead / len(main)
        done = i = 0
        for k, fn in enumerate(main):
            fn()
            start = total * lead * k / len(main)
            while i < len(side) and done + side[i][1] / 2 <= start + step:
                self.phase = min(max((done - start) / max(step, 1), 0), 1)
                side[i][0]()
                done += side[i][1]
                i += 1
        run(side[i:])


def kernel(x_hbm, wqkv_hbm, wo_hbm, w1_hbm, w2_hbm, out_hbm,
           x_s, h_s, raw_s, raw1_s, wk_s, wq_s, wv_s, wo_s, w1_s, w2_s,
           q_s, k_s, v_s, p_s, o_s, t_s, pad_s,
           x_sem, raw_sem, w_sem, out_sem, a_s, b_s):
    tune = TUNE
    hold = Pace()
    interleave = hold.interleave

    def x_copy(b):
        rows = pl.ds(b * TM, TM)
        return pltpu.make_async_copy(x_hbm.at[rows], x_s.at[rows], x_sem.at[b])

    def raw_copy(m, tiles, sem, rows=slice(None)):
        return pltpu.make_async_copy(
            wqkv_hbm.at[pl.ds(*tiles), rows, pl.ds(D * (1, 0, 2)[m], D)],
            raw_s.at[pl.ds(8 * m + tiles[0], tiles[1]), rows], raw_sem.at[sem])

    def w1_copy(lo, hi):
        cols = (slice(None), pl.ds(512 * lo, 512 * (hi - lo)))
        return pltpu.make_async_copy(w1_hbm.at[cols], raw1_s.at[cols], w_sem.at[lo])

    def out_copy(row, rows, half, sem):
        idx = (pl.ds(row, rows), pl.ds(512 * half, 512))
        return pltpu.make_async_copy(x_s.at[idx], out_hbm.at[idx], out_sem.at[sem])

    def wait(*copies, start=()):
        def go(n):
            for k, c in enumerate(start):
                pl.when(n == k)(c.start)
            for c in copies:
                pl.when(n == len(start))(c.wait)
        hold.reset(each(0, max(len(start) + 1, 2), go))

    def rhs_square(sp, load, put):
        return [x for ka in range(sp.sub) for na in range(sp.sub) for x in staged(
            emit_forms(False, sp.n,
                       lambda r, c, ka=ka, na=na: hold(load(
                           sp.tile(r, ka), sp.tile(c, na))).astype(F32),
                       lambda i, val, ka=ka, na=na: put(i, ka, na, val)),
            form_costs(sp.n, 4))]

    def proj_square(w_s, kc, s, a, load):
        def put(i, ka, na, val):
            w_s[i, 2 * a + na, pl.ds(128 * (2 * kc + ka) + 16 * s, 16), :] = val
        return rhs_square(ONE, load, put)

    def prep_qkv(m, w_s, halves=(0, 1), slabs=range(8), later=None):
        def permute(kc, s, r):
            w = cat([pltpu.bitcast(raw_s[8 * m + 4 * kc + r + e, pl.ds(16 * s, 16), :], U32)
                     for e in range(2)], 0)
            xs = skew([tile(w, t) for t in range(8)], 4, 1)
            yield
            xs = unskew(xs, 4, 1)
            yield
            for c, x in enumerate(xs):
                p_s[c, pl.ds(256 * kc + 32 * s + 8 * r, 16), :] = pltpu.bitcast(x, F32)

        tasks = []
        for kc in halves:
            pieces = []
            for s in slabs:
                for a in range(2):
                    x, y, z = staged(permute(kc, s, 2 * a), [32, 52, 16])
                    square = proj_square(
                        w_s, kc, s, a, lambda r, c, s=s, a=a, kc=kc: pltpu.bitcast(
                            p_s[4 * a + c, pl.ds(256 * kc + 32 * s + 8 * r, 8), :], BF))
                    if a and later is not None:
                        later += square
                        square = []
                    pieces.append([[x], [], [], [y], [], [], [z], [], square])
            tasks += diagonal(pieces)
        return tasks

    def prep_wo():
        tasks = []
        for kc in range(2):
            for s in range(8):
                for a in range(2):
                    rows = []

                    def fetch(kc=kc, s=s, a=a, rows=rows):
                        hh, t2 = divmod(s, 2)
                        rows.extend(unskew(skew([pltpu.bitcast(raw_s[
                            28 + 4 * t2 + t, pl.ds(32 * hh + 16 * kc, 16),
                            pl.ds(512 * a, 512)], U32) for t in range(4)], 2, 0), 2, 0))
                    tasks.append((fetch, 70))
                    tasks += proj_square(
                        wo_s, kc, s, a,
                        lambda r, c, rows=rows: pltpu.bitcast(tile(rows[r], c), BF))
        return tasks

    def prep_w1(j):
        def square(kc, s):
            def put(i, ka, na, val):
                w1_s[j, i, 0, pl.ds(128 * kc + 16 * s, 16), :] = val
            return rhs_square(TWO, lambda r, c: raw1_s[
                pl.ds(512 * kc + 128 * r + 16 * s, 16), pl.ds(512 * j + 128 * c, 128)], put)
        return [x for kc in range(2) for s in range(8) for x in square(kc, s)]

    def prep_w2(j):
        def square(a, s):
            def put(i, ka, na, val):
                w2_s[j, i, a, pl.ds(16 * s, 16), :] = val
            return rhs_square(TWO, lambda r, c: raw_s[
                4 * j + r, pl.ds(16 * s, 16), pl.ds(512 * a + 128 * c, 128)], put)
        return [x for a in range(2) for s in range(8) for x in square(a, s)]

    def moments(load, out):
        x = [load(j) for j in range(8)]
        mean = jnp.sum(functools.reduce(jnp.add, x), axis=-1, keepdims=True) * (1.0 / D)
        yield
        x = [t - mean for t in x]
        sq = functools.reduce(jnp.add, [t * t for t in x])
        var = jnp.sum(sq, axis=-1, keepdims=True) * (1.0 / D)
        yield
        inv = lax.rsqrt(var + EPS)
        out.append(lambda j: hold(x[j]) * inv)

    def norm(sp, load, dst, first_cost):
        stats, forms = [], []
        for t in range(sp.slabs):
            rows = [[] for _ in range(sp.n)]
            stats.append(merge(*[staged(moments(
                functools.partial(load, 16 * sp.slab(g, t)), rows[g]), [first_cost, 46, 10])
                for g in range(sp.n)]))

            def put(i, val, a, t=t):
                dst[i, a, pl.ds(16 * t, 16), :] = val
            forms.append([x for a in range(8 // sp.n) for x in staged(
                emit_forms(True, sp.n,
                           lambda r, c, a=a, rows=rows: rows[r][0](sp.tile(c, a)),
                           functools.partial(put, a=a)),
                form_costs(sp.n, 4))])
        return stats, forms

    def norm1(row0, dst):
        return norm(ONE, lambda r, j: hold(
            x_s[pl.ds(row0 + r, 16), pl.ds(128 * j, 128)]).astype(F32), dst, 38)

    def norm2(row0):
        return norm(TWO, lambda r, j: hold(h_s[j, pl.ds(row0 + r, 16), :]), b_s, 30)

    def project(lhs_s, w_s, sink, halves=False, park=True):
        stages, early = [], []
        for a0 in (0, 2):
            for r in range(2):
                m = {}

                def dot(i, k, a0=a0, r=r, m=m):
                    d = mm(cat([lhs_s.bitcast(U32)[i, 2 * k + c, pl.ds(64 * r, 64), :]
                                for c in range(2)], 1),
                           cat([w_s.bitcast(U32)[i, a0 + a, pl.ds(128 * k, 128), :]
                                for a in range(2)], 1))
                    hold.mark(tile(d, 0))
                    for a in range(2):
                        n = ((a0 + a) * 7 + i) * 256 + 128 * r
                        spot = (n // S, pl.ds(n % S, 128))
                        if halves and park and k == 0:
                            h_s[spot] = tile(d, a)
                        elif halves and park:
                            m[a, i] = h_s[spot] + tile(d, a)
                        else:
                            m[a, i] = tile(d, a) if k == 0 else m[a, i] + tile(d, a)

                def post(t, a, a0=a0, r=r, m=m):
                    c = yield from out_forms(lambda i: m[a, i][16 * t:16 * t + 16], 0, 7)
                    for g in range(2):
                        for cc in range(2):
                            sink(ONE.tile(cc, a0 + a), ONE.slab(g, 8 * r + t), c[g][cc])

                posts = [x for a in range(2) for t in range(8)
                         for x in staged(post(t, a), [18, 10])]
                if halves:
                    early.append(([functools.partial(dot, i, 0) for i in range(7)], []))
                stages.append(([functools.partial(dot, i, k) for i in range(7)
                                for k in ((1,) if halves else (0, 1))], posts))
        return (early, stages) if halves else stages

    def run_stages(stages, carried, side, lead=1.0):
        idle = sum(c for _, c in side) * (lead - 1)
        side = side + [(lambda: None, idle / 8)] * 8
        for (dots, posts), part in zip(stages, split(side, len(stages))):
            interleave(dots, carried + part)
            carried = posts
        return carried

    def to_ref(ref, off):
        def sink(j, sl, val):
            ref[j, pl.ds(off + 16 * sl, 16), :] = val
        return sink

    def residual(row0):
        def sink(j, sl, val):
            rows = pl.ds(row0 + 16 * sl, 16)
            h_s[j, rows, :] = hold(x_s[rows, pl.ds(128 * j, 128)]).astype(F32) + val
        return sink

    def scores(first_block):
        lane = lax.broadcasted_iota(jnp.int32, (8, 128), 1)
        odd, high = (lane & 1) != 0, (lane & 2) != 0
        up = lambda x, b: pltpu.roll(x, b, 1)
        down = lambda x, b: pltpu.roll(x, 128 - b, 1)

        def go(r):
            acc = [None] * WIN
            for j in range(8):
                q = hold(q_s[j, pl.ds(r, 8), :])
                for w in range(WIN):
                    kw = k_s[j, pl.ds(HALO + r - DIL * w, 8), :]
                    acc[w] = q * kw if j == 0 else acc[w] + q * kw
                if j % 2:
                    yield
            xs = [(acc[w], up(acc[w], 1), acc[w + 1], down(acc[w + 1], 1))
                  for w in range(0, WIN, 2)]
            yield
            xs = [jnp.where(odd, a + ua, b + db) for a, ua, b, db in xs]
            xs = [hold(x) for x in xs]
            xs = [(x, up(x, 2), down(x, 2)) for x in xs]
            yield
            logit = [x + jnp.where(high, u, d) for x, u, d in xs]
            if first_block and r < DIL * (WIN - 1):
                row = lax.broadcasted_iota(jnp.int32, (8, 128), 0) + r
                for n, s in enumerate(logit):
                    w = jnp.where(odd, 2 * n, 2 * n + 1)
                    logit[n] = jnp.where(row >= DIL * w, s * SCALE, -1e9)
                factor = LOG2E
            else:
                factor = SCALE * LOG2E
            top = functools.reduce(jnp.maximum, logit)
            u, d = up(top, 1), down(top, 1)
            yield
            top = jnp.maximum(top, jnp.where(odd, u, d))
            e = [jnp.exp2((s - top) * factor) for s in logit]
            total = functools.reduce(jnp.add, e)
            u, d = up(total, 1), down(total, 1)
            yield
            inv = 1.0 / (total + jnp.where(odd, u, d))
            e = [x * inv for x in e]
            xs = [(x, up(x, 1), down(x, 1)) for x in e]
            yield
            e = [y for x, u, d in xs for y in (jnp.where(odd, x, d), jnp.where(odd, u, x))]
            for w in range(WIN):
                p_s[w, pl.ds(r, 8), :] = e[w]

        pieces = [staged(go(r), [32] * 4 + [8, 20, 12, 16, 16, 16]) for r in range(0, TM, 8)]
        return [task for n in range(len(pieces) + 6) for task in merge(
            pieces[n][:4] if n < len(pieces) else [],
            [pieces[n - k][3 + k] for k in range(1, 7) if 0 <= n - k < len(pieces)])]

    def mix(dst):
        def go(t, a):
            grid = [[], []]
            for g in range(2):
                r = 16 * ONE.slab(g, t)
                p = [hold(p_s[w, pl.ds(r, 16), :]) for w in range(WIN)]
                for c in range(2):
                    terms = []
                    for w in range(WIN // 2):
                        v = v_s[ONE.tile(c, a), pl.ds(HALO + r - DIL * w - 8, 24), :]
                        terms.append(p[w] * v[8:] + p[w + 4] * v[:16])
                    grid[g].append((terms[0] + terms[1]) + (terms[2] + terms[3]))
                    yield

            def put(i, val):
                dst[i, a, pl.ds(16 * t, 16), :] = val
            yield from emit_forms(True, 2, lambda g, c: grid[g][c], put)

        return [x for lo in (0, 2) for t in range(ONE.slabs) for a in (lo, lo + 1)
                for x in staged(go(t, a), [46, 30, 46, 30, 17])]

    def halo(ref):
        def keep():
            ref[:, pl.ds(0, HALO), :] = ref[:, pl.ds(TM, HALO), :]
        return [(keep, 0)]

    def first_halo():
        for j in range(8):
            v_s[j, pl.ds(0, HALO), :] = jnp.broadcast_to(
                v_s[j, pl.ds(HALO, 1), :], (HALO, 128))

    def expand():
        stages = []
        for j in range(NCH):
            m = [None] * TWO.p

            def dot(p, j=j, m=m):
                m[p] = mm(cat([b_s.bitcast(U32)[p, c] for c in range(2)], 1),
                          w1_s.bitcast(U32)[j, p, 0])
                hold.mark(m[p])

            def post(t, j=j, m=m):
                c = yield from out_forms(lambda p: m[p][16 * t:16 * t + 16], 0, TWO.p)

                def put(p, val):
                    t_s[p, j, pl.ds(16 * t, 16), :] = val
                yield from emit_forms(True, 4, lambda g, cc: silu(hold(c[g][cc])), put)

            stages.append(([functools.partial(dot, p) for p in range(TWO.p)],
                           [x for t in range(TWO.slabs) for x in staged(
                               post(t), [0] * 7 + form_costs(4, tune["silu_cost"]))]))
        return stages

    def parked(p, rows=slice(None)):
        ref, start = (q_s, p_s)[p // 32], 128 * (p % 4)
        lo, hi, _ = rows.indices(128)
        return ref, (p % 32 // 4, pl.ds(start + lo, hi - lo))

    def contract(row0, a):
        m = [None] * TWO.p

        def dot(p, j0, j1):
            d = mm(cat([t_s.bitcast(U32)[p, j] for j in range(j0, j1)], 1),
                   cat([w2_s.bitcast(U32)[j, p, a] for j in range(j0, j1)], 0))
            m[p] = d if m[p] is None else m[p] + d
            hold.mark(d)
            if a and j1 == NCH:
                ref, idx = parked(p)
                ref[idx] = m[p]

        def product(p, t):
            if not a:
                return m[p][16 * t:16 * t + 16]
            ref, idx = parked(p, slice(16 * t, 16 * t + 16))
            return hold(ref[idx])

        def post(t):
            c = yield from out_forms(lambda p: product(p, t), 0, TWO.p)
            for g in range(4):
                rows = pl.ds(row0 + 16 * TWO.slab(g, t), 16)
                x_s[rows, pl.ds(512 * a, 512)] = cat(
                    [h_s[4 * a + cc, rows, :] + (c[g][cc] if a else hold(c[g][cc]))
                     for cc in range(4)], 1).astype(BF)
                if g == 1:
                    yield

        def dots(products, *edges):
            return [functools.partial(dot, p, j0, j1) for p in products
                    for j0, j1 in zip(edges, edges[1:])]

        posts = [x for t in range(TWO.slabs)
                 for x in staged(post(t), [30 if a else 0] * 7 + [36] * 2)]
        if a:
            return [(dots(range(TWO.p), 0, 2, 4, NCH), posts)]
        n = tune["early_products"]
        return [(dots(range(n), 0, 2, 4, NCH - 1), []),
                (dots(range(n), NCH - 1, NCH) + dots(range(n, TWO.p), 0, 2, 4, NCH), posts)]

    k_stages = lambda lhs, **kw: project(lhs, wk_s, to_ref(k_s, HALO), **kw)
    q_stages = lambda lhs, **kw: project(lhs, wq_s, to_ref(q_s, 0), **kw)
    v_stages = lambda lhs: project(lhs, wv_s, to_ref(v_s, HALO))
    o_stages = lambda b, lhs, **kw: project(lhs, wo_s, residual(b * TM), **kw)
    flat = lambda parts: [x for part in parts for x in part]
    lead, q_lead, v_lead = tune["lead"], tune["q_lead"], tune["v_lead"]

    jobs = [f(j) for f in (prep_w1, prep_w2) for j in range(NCH)]
    take = lambda n: flat([jobs.pop(0) for _ in range(n)])
    first_stats, first_forms = (flat(x) for x in norm2(0))

    head = [raw_copy(0, (0, 4), h, pl.ds(64 * h, 64)) for h in range(2)]
    k1 = [raw_copy(0, (4, 4), 2 + 7 * h, pl.ds(64 * h, 64)) for h in range(2)]
    q0, q1, v0, v1 = (raw_copy(m, (4 * kc, 4), 2 * m + kc + 1)
                      for m in (1, 2) for kc in range(2))
    x0 = [pltpu.make_async_copy(x_hbm.at[pl.ds(256 * r, 256)], x_s.at[pl.ds(256 * r, 256)],
                                x_sem.at[NB * r]) for r in range(2)]
    wo = pltpu.make_async_copy(wo_hbm, raw_s.at[pl.ds(28, 8)], raw_sem.at[7])
    w1 = [w1_copy(0, 1), w1_copy(1, 2), w1_copy(2, NCH)]
    w2 = pltpu.make_async_copy(w2_hbm, raw_s.at[pl.ds(0, 28)], w_sem.at[3])
    fence = pltpu.make_async_copy(wo_hbm.at[0, pl.ds(0, 16)], pad_s, raw_sem.at[8])

    wait(x0[0], start=[x0[0], *head, x0[1], *k1, q0, q1, v0, x_copy(1), v1,
                       wo, x_copy(2), w1[0]])
    k_s[:, pl.ds(0, HALO), :] = jnp.zeros((8, HALO, 128), F32)
    stats, forms = norm1(0, o_s)
    run(overlap(stats[:8], forms[:8]))
    right = []
    for h in range(2):
        wait(head[h])
        run(prep_qkv(0, wk_s, (0,), range(4 * h, 4 * h + 4), right))
    early, late = k_stages(o_s, halves=True)
    dots = flat(early[n][0] for n in (0, 2, 1, 3))
    n0, n1, n2 = tune["head_cuts"]
    interleave(dots[:n0], right, lead=1.0)
    x0[1].wait()
    interleave(dots[n0:n1], overlap(stats[8:], forms[8:]), lead=1.0)
    for h, part in enumerate((dots[n1:n2], dots[n2:])):
        k1[h].wait()
        interleave(part, prep_qkv(0, wk_s, (1,), range(4 * h, 4 * h + 4)), lead=1.0)
    run([(d, 0) for st in late[:2] for d in st[0]])
    q0.wait()
    left = run_stages(late[2:], flat(st[1] for st in late[:2]), prep_qkv(1, wq_s, (0,)), q_lead)
    wait(q1)
    early, late = q_stages(o_s, halves=True)
    run_stages(early, left, prep_qkv(1, wq_s, (1,)), q_lead)
    wait(v0, x_copy(1))
    stats, forms = (flat(x) for x in norm1(TM, a_s))
    left = run_stages(late, [], merge(prep_qkv(2, wv_s, (0,)), stats), v_lead)
    wait(v1, start=[w1[1], w1[2]])
    early, late = project(o_s, wv_s, to_ref(v_s, HALO), halves=True, park=False)
    sc_a, sc_b = cut(scores(True), tune["first_scores"])
    forms_a, forms_b = cut(forms, tune["early_forms"])
    run_stages(early, left, merge(prep_qkv(2, wv_s, (1,)), forms_a), v_lead)
    left = run_stages(late, [], merge(sc_a, forms_b), tune["first_lead"])

    for b in range(1, NB):
        last = b == NB - 1
        nk, nq, nv, no = tune["weights"][4 * b - 4:4 * b]
        mix_a, mix_b = cut(mix(o_s), 0.0 if b == 1 else tune["mix"])
        if b == 1:
            wait(wo, x_copy(2), w1[0], start=[w2, x_copy(3), fence])
            stages = k_stages(a_s)
            interleave(flat(st[0] for st in stages[:2]), merge(left, sc_b), lead=1.1)
            left = [(first_halo, 0)] + halo(k_s) + flat(st[1] for st in stages[:2])
            left = run_stages(stages[2:], left, prep_wo() + take(nk))
        else:
            left = run_stages(k_stages(a_s), halo(k_s) + left, merge(mix_a, take(nk)))
        if b == 2:
            wait(w2, x_copy(3))
        left = run_stages(q_stages(a_s), left, merge(mix_b, take(nq)), lead)
        if b == 1:
            wait(w1[1], w1[2])
        if last:
            wait(fence)
        sc_a, sc_b = cut(scores(False), tune["last_scores" if last else "scores"])
        stats, forms = ([], []) if last else (flat(x) for x in norm1((b + 1) * TM, a_s))
        left = run_stages(v_stages(a_s), halo(v_s) + left, merge(sc_a, stats, take(nv)))
        if not last:
            left = run_stages(o_stages(b - 1, o_s), left, merge(
                sc_b, forms, first_stats if b == 2 else [], take(no)), lead)
    mix_a, mix_b = cut(mix(a_s), tune["last_mix"])
    forms_a, forms_b = cut(first_forms, tune["first_forms"])
    left = run_stages(o_stages(NB - 2, o_s), left,
                      merge(sc_b + merge(mix_a, forms_a), take(no)), lead)
    early, late = o_stages(NB - 1, a_s, halves=True, park=False)
    run_stages(early, left, merge(mix_b, forms_b, take(tune["weights"][-2])), lead)
    run(run_stages(late, [], take(tune["weights"][-1]), lead))
    assert not jobs

    def ffn_step(i, carry):
        row0 = pl.multiple_of(i * TM, TM)
        nxt = pl.multiple_of(jnp.minimum(i + 1, NB - 1) * TM, TM)
        prev = pl.multiple_of((i + NB - 1) % NB * TM, TM)
        hold.reset(i)
        left = run_stages(expand(), contract(prev, 1)[0][1], [])
        one, two = contract(row0, 0)
        interleave(one[0], left)
        norm_a, norm_b = cut(flat(flat(x) for x in norm2(nxt)), tune["norm"])
        left = run_stages([two], [], norm_a)
        dots = contract(row0, 1)[0][0]
        n = int(TWO.p * tune["send"]) * 3
        interleave(dots[:n], merge(left, norm_b), lead=tune["out_lead"])

        def send(k):
            pl.when(k == 1)(out_copy(row0, TM, 0, 2 * i).start)
            pl.when(k == 0)(out_copy(prev, TM, 1, jnp.maximum(2 * i - 1, 0)).start)
        each(jnp.where(i > 0, 0, 1), 2, send)
        run([(d, 0) for d in dots[n:]])
        return carry

    lax.fori_loop(0, NB, ffn_step, 0)
    hold.latest = None
    tail = [out_copy(S - TM + 128 * u, 128, 1, 2 * NB - 1 + u) for u in range(4)]
    for tasks, c in zip(split(contract(S - TM, 1)[0][1], 4), tail):
        run(tasks)
        c.start()
    for c in [out_copy(n // 2 * TM, TM, n % 2, n) for n in range(2 * NB - 1)] + tail:
        c.wait()


@jax.jit
def pallas_sequential_preLN__sliding_local_dilated__dense_activation_silu__prompt_kernel(
    A_x: jax.Array,
    A_wqkv: jax.Array,
    A_wo: jax.Array,
    B_x: jax.Array,
    B_w1: jax.Array,
    B_w2: jax.Array,
):
    del B_x
    scratch = [
        pltpu.VMEM((S, D), BF),
        pltpu.VMEM((8, S, 128), F32),
        pltpu.VMEM((36, 128, D), BF),
        pltpu.VMEM((D, F), BF),
        pltpu.VMEM(ONE.forms(D, D), BF),
        pltpu.VMEM(ONE.forms(D, D), BF),
        pltpu.VMEM(ONE.forms(D, D), BF),
        pltpu.VMEM(ONE.forms(D, D), BF),
        pltpu.VMEM((NCH,) + TWO.forms(D, 512), BF),
        pltpu.VMEM((NCH,) + TWO.forms(512, D), BF),
        pltpu.VMEM((8, TM, 128), F32),
        pltpu.VMEM((8, HALO + TM, 128), F32),
        pltpu.VMEM((8, HALO + TM, 128), F32),
        pltpu.VMEM((WIN, TM, 128), F32),
        pltpu.VMEM(ONE.forms(TM, D), BF),
        pltpu.VMEM(TWO.forms(TM, F), BF),
        pltpu.VMEM((16, D), BF),
        pltpu.SemaphoreType.DMA((NB + 1,)),
        pltpu.SemaphoreType.DMA((10,)),
        pltpu.SemaphoreType.DMA((4,)),
        pltpu.SemaphoreType.DMA((2 * NB + 3,)),
        pltpu.VMEM(ONE.forms(TM, D), BF),
        pltpu.VMEM(TWO.forms(TM, D), BF),
    ]
    out = pl.pallas_call(
        kernel,
        in_specs=[pl.BlockSpec(memory_space=pl.ANY)] * 5,
        out_specs=pl.BlockSpec(memory_space=pl.ANY),
        out_shape=jax.ShapeDtypeStruct((S, D), BF),
        scratch_shapes=scratch,
        compiler_params=pltpu.CompilerParams(vmem_limit_bytes=126 << 20),
    )(A_x.reshape(S, D), A_wqkv.reshape(8, 128, 3 * D), A_wo.reshape(8, 128, D),
      B_w1, B_w2.reshape(F // 128, 128, D))
    return out.reshape(1, S, D)
```
